```python
import jax
import jax.numpy as jnp

def _softmax(x, axis=-1):
    return jax.nn.softmax(x, axis=axis)

def _gelu(x):
    return jax.nn.gelu(x, approximate=True)

def _silu(x):
    return jax.nn.silu(x)

def _sigmoid(x):
    return jax.nn.sigmoid(x)

def _layernorm(x, axis=-1, eps=1e-05):
    m = jnp.mean(x, axis=axis, keepdims=True)
    v = jnp.var(x, axis=axis, keepdims=True)
    return (x - m) / jnp.sqrt(v + eps)

def _scatter_add(tgt, idx, src, axis=0):
    return tgt.at[idx].add(src)

def _segment_sum(src, seg, n):
    return jax.ops.segment_sum(src, seg, n)

class _Rng:

    def __init__(self, key):
        self._k = key

    def _next(self):
        self._k, sub = jax.random.split(self._k)
        return sub

    def normal(self, shape):
        return jax.random.normal(self._next(), shape, dtype=jnp.bfloat16)

    def randint(self, lo, hi, shape):
        return jax.random.randint(self._next(), shape, lo, hi, dtype=jnp.int32)

    def uniform(self, shape, lo=0.0, hi=1.0):
        return jax.random.uniform(self._next(), shape, jnp.bfloat16, lo, hi)

    def permutation(self, n):
        return jax.random.permutation(self._next(), n)
kernel_name = 'interleave_layers__memory_aug_recurrent_mem_tr__spectral_gfnet__prompt'

def setup_inputs():
    _rng = _Rng(jax.random.key(int.from_bytes(__import__("os").urandom(4), "little")))
    _w = lambda a: (lambda t: t.astype(jnp.bfloat16) if jnp.issubdtype(t.dtype, jnp.floating) else t)(jnp.asarray(a))

    def _A_setup():
        B, S, Dm = (1, 2048, 640)
        H, Dh = (32, 128)
        M, seg = (8, 32)
        seg = min(seg, S)
        S = S // seg * seg
        return {'x': _w((lambda *s: _rng.normal(s) * 0.05)(B, S, Dm)), 'mem0': _w((lambda *s: _rng.normal(s) * 0.05)(B, M, Dm)), 'Wq': _w((lambda *s: _rng.normal(s) * 0.05)(Dm, H, Dh) * Dm ** (-0.5)), 'Wk': _w((lambda *s: _rng.normal(s) * 0.05)(Dm, H, Dh) * Dm ** (-0.5)), 'Wv': _w((lambda *s: _rng.normal(s) * 0.05)(Dm, H, Dh) * Dm ** (-0.5)), 'Wo': _w((lambda *s: _rng.normal(s) * 0.05)(H, Dh, Dm) * (H * Dh) ** (-0.5)), 'seg_len': seg}
    _A_in = _A_setup()

    def _B_setup():
        B, S, D = (1, 2048, 640)
        Df = D // 2 + 1
        return {'x': _w((lambda *s: _rng.normal(s) * 0.05)(B, S, D)), 'w_r': _w((lambda *s: _rng.normal(s) * 0.05)(S, Df) * 0.02), 'w_i': _w((lambda *s: _rng.normal(s) * 0.05)(S, Df) * 0.02)}
    _B_in = _B_setup()
    return {'A_x': _A_in['x'], 'A_mem0': _A_in['mem0'], 'A_Wq': _A_in['Wq'], 'A_Wk': _A_in['Wk'], 'A_Wv': _A_in['Wv'], 'A_Wo': _A_in['Wo'], 'A_seg_len': _A_in['seg_len'], 'B_x': _B_in['x'], 'B_w_r': _B_in['w_r'], 'B_w_i': _B_in['w_i']}

def reference(A_x, A_mem0, A_Wq, A_Wk, A_Wv, A_Wo, A_seg_len, B_x, B_w_r, B_w_i):

    def _A_ref(x, mem0, Wq, Wk, Wv, Wo, seg_len):
        B, S, Dm = x.shape
        H, Dh = (Wq.shape[1], Wq.shape[2])
        M = mem0.shape[1]
        scale = Dh ** (-0.5)
        n_seg = S // seg_len
        L = M + seg_len
        idx = jnp.arange(L)
        mask = (idx[:, None] < M) | (idx[:, None] >= idx[None, :])
        mem = mem0
        outs = []
        for s in range(n_seg):
            xs = x[:, s * seg_len:(s + 1) * seg_len, :].copy()
            h = jnp.concatenate([mem, xs], axis=1)
            q = jnp.einsum('btd,dhe->bhte', h, Wq)
            k = jnp.einsum('btd,dhe->bhte', h, Wk)
            v = jnp.einsum('btd,dhe->bhte', h, Wv)
            scores = jnp.einsum('bhqe,bhke->bhqk', q, k) * scale
            scores = jnp.where(mask[None, None], scores, -1000000000.0)
            p = _softmax(scores, axis=-1)
            o = jnp.einsum('bhqk,bhke->bhqe', p, v)
            o = jnp.einsum('bhte,hed->btd', o, Wo)
            mem = o[:, :M, :].copy()
            outs.append(o[:, M:, :])
        return jnp.concatenate(outs, axis=1)

    def _B_ref(x, w_r, w_i):
        B, S, D = x.shape
        X = (lambda x, axes=(-2, -1): jnp.fft.rfft2(x.astype(jnp.float32), axes=axes))(x, axes=(-2, -1))
        W = w_r + 1j * w_i
        X = X * W
        y = (lambda x, s, axes=(-2, -1): jnp.fft.irfft2(x, s=s, axes=axes).astype(jnp.bfloat16))(X, (S, D), axes=(-2, -1))
        return y
    x = A_x
    x = x + _A_ref(_layernorm(x, axis=-1), A_mem0, A_Wq, A_Wk, A_Wv, A_Wo, A_seg_len)
    x = x + _B_ref(_layernorm(x, axis=-1), B_w_r, B_w_i)
    x = x + _A_ref(_layernorm(x, axis=-1), A_mem0, A_Wq, A_Wk, A_Wv, A_Wo, A_seg_len)
    x = x + _B_ref(_layernorm(x, axis=-1), B_w_r, B_w_i)
    return x
```

```python
import functools

import jax
import jax.numpy as jnp
import numpy as np
import jax.experimental.pallas as pl
import jax.experimental.pallas.tpu as pltpu

F32, BF16, U32 = jnp.float32, jnp.bfloat16, jnp.uint32
LANE = 128
R = 16


def _dot(a, b):
    return jax.lax.dot_general(a, b, (((1,), (0,)), ((), ())), preferred_element_type=F32)


def _dot_nt(a, b):
    return jax.lax.dot_general(a, b, (((1,), (1,)), ((), ())), preferred_element_type=F32)


def _layernorm(x):
    inv = 1.0 / x.shape[-1]
    c = x - jnp.sum(x, axis=-1, keepdims=True) * inv
    v = jnp.sum(c * c, axis=-1, keepdims=True) * inv
    return c * jax.lax.rsqrt(v + 1e-5)


def _dft_constants(S, D, FP):
    nf = D // 2 + 1
    d = np.arange(D)[:, None]
    k = np.arange(nf)[None, :]
    ang = 2.0 * np.pi * ((d * k) % D) / D
    cos, sin = np.cos(ang), np.sin(ang)
    sin[:, 0] = 0.0
    sin[:, D // 2] = 0.0
    fwd = np.zeros((D, 2 * FP))
    fwd[:, :nf] = cos
    fwd[:, FP:FP + nf] = -sin
    ck = np.full((nf,), 2.0)
    ck[0] = ck[D // 2] = 1.0
    inv = np.zeros((2 * FP, D))
    inv[:nf] = (cos * ck / D).T
    inv[FP:FP + nf] = (-sin * ck / D).T
    k1 = np.arange(R)[:, None, None]
    k2 = np.arange(LANE)[None, :, None]
    n2 = np.arange(LANE)[None, None, :]
    a = 2.0 * np.pi * ((n2 * (k1 + R * k2)) % S) / S
    c, s = np.cos(a), np.sin(a)
    g = np.concatenate([np.concatenate([c, s], 2), np.concatenate([-s, c], 2)], 1)
    gi = np.transpose(g, (0, 2, 1)) / S
    slab = lambda m: np.ascontiguousarray(
        m.reshape(m.shape[0], -1, LANE).transpose(1, 0, 2)).astype(BF16)
    return slab(fwd), slab(inv), g.astype(BF16), gi.astype(BF16)


def _fft4(x, sign):
    (ar, ai), (br, bi), (cr, ci), (dr, di) = x
    sr, si, tr, ti = ar + cr, ai + ci, ar - cr, ai - ci
    ur, ui, vr, vi = br + dr, bi + di, br - dr, bi - di
    p, m = (tr - vi, ti + vr), (tr + vi, ti - vr)
    y1, y3 = (p, m) if sign > 0 else (m, p)
    return [(sr + ur, si + ui), y1, (sr - ur, si - ui), y3]


def _twiddle16(z, e, sign):
    r, i = z
    if e == 0:
        return z
    if e == 4:
        return (-i, r) if sign > 0 else (i, -r)
    c = float(np.cos(2 * np.pi * e / 16))
    s = float(sign * np.sin(2 * np.pi * e / 16))
    if e % 4 == 2:
        sg = s / c
        return ((r - i) * c, (i + r) * c) if sg > 0 else ((r + i) * c, (i - r) * c)
    return (r * c - i * s, i * c + r * s)


def _fft16(x, sign):
    t = [_fft4([x[b + 4 * a] for a in range(4)], sign) for b in range(4)]
    y = [None] * 16
    for k1 in range(4):
        o = _fft4([_twiddle16(t[b][k1], b * k1, sign) for b in range(4)], sign)
        for k2 in range(4):
            y[k1 + 4 * k2] = o[k2]
    return y


def _kernel(x_hbm, mem_hbm, wq_hbm, wk_hbm, wv_hbm, wo_hbm, wr_hbm, wi_hbm,
            fd_hbm, fi_hbm, g_hbm, gi_hbm, out_hbm,
            xb, mem0, stage, wqkv, wo, wrb, wib, wrf, wif, fd, fi, g, gi,
            x, hbuf, oc, otok, fill, xa, ya, sems, *, S, D, H, M, SEG, FP):
    L = M + SEG
    nseg = S // SEG
    ND = D // LANE
    NF = FP // LANE
    nf = D // 2 + 1
    G = LANE // L
    groups = [list(range(a, min(a + G, H))) for a in range(0, H, G)]
    scale = LANE ** -0.5
    CH = 256

    rows = LANE * H // 2
    cp_x = pltpu.make_async_copy(x_hbm, xb, sems.at[0])
    cp_mem = pltpu.make_async_copy(mem_hbm, mem0, sems.at[1])
    cp_w = [pltpu.make_async_copy(w.bitcast(U32).at[pl.ds(c * rows, rows)], stage.at[i * ND + c],
                                  sems.at[2 + i * ND + c])
            for i, w in enumerate((wq_hbm, wk_hbm, wv_hbm)) for c in range(ND)]
    n = 2 + 3 * ND
    cp_wo = [pltpu.make_async_copy(wo_hbm.at[:, pl.ds(c * LANE, LANE)], wo.at[c], sems.at[n + c])
             for c in range(ND)]
    n += ND
    cp_b = [pltpu.make_async_copy(a, b, sems.at[n + i]) for i, (a, b) in enumerate(
        ((wr_hbm, wrb), (wi_hbm, wib), (fd_hbm, fd), (fi_hbm, fi), (g_hbm, g), (gi_hbm, gi)))]
    n_out = n + len(cp_b)
    for cp in [cp_x, cp_mem] + cp_w + cp_wo:
        cp.start()

    r = jax.lax.broadcasted_iota(jnp.int32, fill.shape, 0)
    c = jax.lax.broadcasted_iota(jnp.int32, fill.shape, 1)
    rb = sum((r >= L * j).astype(jnp.int32) for j in range(1, G + 1))
    cb = sum((c >= L * j).astype(jnp.int32) for j in range(1, G + 1))
    ri, ci = r - L * rb, c - L * cb
    fill[...] = jnp.where(rb == cb, jnp.where((ri < M) | (ri >= ci), 0.0, -1e9),
                          -jnp.inf).astype(F32)
    otok[...] = jnp.zeros(otok.shape, F32)

    cp_x.wait()

    @pl.loop(0, S // CH)
    def _(i):
        r0 = pl.multiple_of(i * CH, CH)
        x[pl.ds(r0, CH), :] = xb[pl.ds(r0, CH), :].astype(F32)

    cp_mem.wait()

    for t, cp in enumerate(cp_w):
        cp.wait()
        i, c = divmod(t, ND)

        @pl.loop(0, H // 2)
        def _(j):
            w = stage[t, pl.ds(j, LANE, stride=H // 2), :]
            lo = pltpu.bitcast(w << 16, F32).astype(BF16)
            hi = pltpu.bitcast(w & np.uint32(0xFFFF0000), F32).astype(BF16)
            wqkv[i * H + 2 * j, c * LANE:(c + 1) * LANE, :] = lo
            wqkv[i * H + 2 * j + 1, c * LANE:(c + 1) * LANE, :] = hi

    for cp in cp_b:
        cp.start()
    for cp in cp_wo:
        cp.wait()

    def finish_segment(s):
        r0 = pl.multiple_of(s * SEG, SEG)
        xn = x[pl.ds(r0, SEG), :] + otok[...]
        x[pl.ds(r0, SEG), :] = xn
        xb[pl.ds(r0, SEG), :] = _layernorm(xn).astype(BF16)

    def a_step(s, carry):
        st = {}

        def proj(i, hd):
            st[i, hd] = _dot(hbuf[...], wqkv[i * H + hd])

        def scores(gi_):
            gr = groups[gi_]
            pad = [jnp.zeros((LANE - L * len(gr), LANE), F32)]
            q = jnp.concatenate([st.pop((0, hd)) for hd in gr], 0)
            k = jnp.concatenate([st.pop((1, hd)) for hd in gr] + pad, 0).astype(BF16)
            st['v', gi_] = jnp.concatenate([st.pop((2, hd)) for hd in gr] + pad, 0).astype(BF16)
            st['s', gi_] = _dot_nt(q, k)

        def softmax(gi_):
            f = fill[0:L * len(groups[gi_]), :]
            sc = jnp.where(f < 0.0, f, st.pop(('s', gi_)) * scale)
            e = jnp.exp(sc - jnp.max(sc, axis=1, keepdims=True))
            st['p', gi_] = e / jnp.sum(e, axis=1, keepdims=True)

        def values(gi_):
            o = _dot(st.pop(('p', gi_)), st.pop(('v', gi_)))
            for j, hd in enumerate(groups[gi_]):
                oc[:, hd * LANE:(hd + 1) * LANE] = o[L * j:L * (j + 1)]
            done.update(groups[gi_])

        def out_proj(h0, h1):
            a, b = h0 * LANE, h1 * LANE
            t = jnp.concatenate([_dot(oc[:, a:b], wo[c, a:b, :]) for c in range(ND)], 1)
            st['acc'] = st['acc'] + t if 'acc' in st else t

        def next_ln(_):
            r1 = pl.multiple_of(jnp.minimum(s + 1, nseg - 1) * SEG, SEG)
            st['ln'] = _layernorm(x[pl.ds(r1, SEG), :])

        def prev_finish(_):
            finish_segment(jnp.maximum(s - 1, 0))

        events, done = {}, set()
        for gi_, gr in enumerate(groups):
            last = 3 * (gr[-1] + 1) - 1
            for delay, fn in ((0, scores), (3, softmax), (9, values)):
                events.setdefault(last + delay, []).append((fn, gi_))
        events.setdefault(0, []).append((prev_finish, 0))
        events.setdefault(3 * H + 16, []).append((next_ln, 0))
        slot = 0

        def tick():
            nonlocal slot
            for fn, a in events.pop(slot, []):
                fn(a)
            slot += 1

        for gr in groups:
            for i in (1, 0, 2):
                for hd in gr:
                    proj(i, hd)
                    tick()
        WC = 4
        for h0 in range(0, H, WC):
            while not done.issuperset(range(h0, h0 + WC)):
                tick()
            out_proj(h0, h0 + WC)
            for _ in range(WC):
                tick()
        assert not events
        hbuf[M:L, :] = st['ln']
        hbuf[0:M, :] = st['acc'][0:M]
        otok[...] = st['acc'][M:L]
        return carry

    def layer_a():
        hbuf[0:M, :] = mem0[...].astype(F32)
        hbuf[M:L, :] = _layernorm(x[0:SEG, :])
        jax.lax.fori_loop(0, nseg, a_step, 0)
        finish_segment(nseg - 1)
        otok[...] = jnp.zeros(otok.shape, F32)

    def radix(src, dst, sign):
        @pl.loop(0, LANE // 8)
        def _(i):
            r0 = pl.multiple_of(i * 8, 8)
            for c in range(NF):
                v = [(src[c, n_, pl.ds(r0, 8), :], src[c, n_, pl.ds(LANE + r0, 8), :])
                     for n_ in range(R)]
                for n_, (re, im) in enumerate(_fft16(v, sign)):
                    dst[c, n_, pl.ds(r0, 8), :] = re
                    dst[c, n_, pl.ds(LANE + r0, 8), :] = im

    def layer_b(layer):
        nb = CH // LANE

        @pl.loop(0, S // CH)
        def _(i):
            xh = xb[pl.ds(pl.multiple_of(i * CH, CH), CH), :]
            for c in range(2 * NF):
                t = _dot(xh, fd[c])
                for j in range(nb):
                    xa[c % NF, i * nb + j, (c // NF) * LANE:(c // NF + 1) * LANE, :] = (
                        t[j * LANE:(j + 1) * LANE])

        radix(xa, ya, -1)

        @pl.loop(0, R)
        def _(k1):
            z = [_dot(g[k1], ya[c, k1].astype(BF16)) for c in range(NF)]
            for c in range(NF):
                zr, zi = z[c][0:LANE], z[c][LANE:]
                wr = wrf[c, pl.ds(k1, LANE, stride=R), :]
                wi = wif[c, pl.ds(k1, LANE, stride=R), :]
                zz = jnp.concatenate([zr * wr - zi * wi, zr * wi + zi * wr], 0).astype(BF16)
                xa[c, k1] = _dot(gi[k1], zz)

        radix(xa, ya, +1)

        def out_copy(i):
            rs = pl.ds(pl.multiple_of(i * CH, CH), CH)
            return pltpu.make_async_copy(xb.at[rs], out_hbm.at[rs], sems.at[n_out + i])

        @pl.loop(0, S // CH)
        def _(i):
            rs = pl.ds(pl.multiple_of(i * CH, CH), CH)
            zz = jnp.concatenate([
                jnp.concatenate([ya[c % NF, i * nb + j, (c // NF) * LANE:(c // NF + 1) * LANE, :]
                                 for j in range(nb)], 0).astype(BF16)
                for c in range(2 * NF)], 1)
            xn = x[rs, :] + jnp.concatenate([_dot(zz, fi[c]) for c in range(ND)], 1)
            x[rs, :] = xn
            xb[rs, :] = xn.astype(BF16)

            @pl.when(layer == 1)
            def _():
                out_copy(i).start()

        @pl.when(layer == 1)
        def _():
            for i in range(S // CH):
                out_copy(i).wait()

    @pl.loop(0, 2)
    def _(layer):
        layer_a()

        @pl.when(layer == 0)
        def _():
            for cp in cp_b:
                cp.wait()
            tail = nf - (NF - 1) * LANE

            @pl.loop(0, S // CH)
            def _(i):
                rs = pl.ds(pl.multiple_of(i * CH, CH), CH)
                for src, dst in ((wrb, wrf), (wib, wif)):
                    for c in range(NF - 1):
                        dst[c, rs, :] = src[rs, c * LANE:(c + 1) * LANE].astype(F32)
                    dst[NF - 1, rs, :] = jnp.concatenate(
                        [src[rs, (NF - 1) * LANE:nf].astype(F32),
                         jnp.zeros((CH, LANE - tail), F32)], 1)

        layer_b(layer)


@functools.partial(jax.jit, static_argnames=("A_seg_len",))
def pallas_interleave_layers__memory_aug_recurrent_mem_tr__spectral_gfnet__prompt_kernel(
    A_x, A_mem0, A_Wq, A_Wk, A_Wv, A_Wo, A_seg_len, B_x, B_w_r, B_w_i,
):
    del B_x
    B, S, D = A_x.shape
    _, H, Dh = A_Wq.shape
    M = A_mem0.shape[1]
    SEG = int(A_seg_len)
    nf = D // 2 + 1
    FP = -(-nf // LANE) * LANE
    L = M + SEG
    assert B == 1 and Dh == LANE and S == R * LANE and D % LANE == 0 and S % SEG == 0
    assert M % 8 == 0 and SEG % 16 == 0 and L <= LANE and H % 4 == 0
    ND, NF = D // LANE, FP // LANE
    consts = _dft_constants(S, D, FP)

    vm = pltpu.VMEM
    scratch = [
        vm((S, D), BF16),
        vm((M, D), BF16),
        vm((3 * ND, LANE * H // 2, LANE), U32),
        vm((3 * H, D, LANE), BF16),
        vm((ND, H * Dh, LANE), BF16),
        vm((S, nf), BF16), vm((S, nf), BF16),
        vm((NF, S, LANE), F32), vm((NF, S, LANE), F32),
        vm(consts[0].shape, BF16), vm(consts[1].shape, BF16),
        vm(consts[2].shape, BF16), vm(consts[3].shape, BF16),
        vm((S, D), F32),
        vm((L, D), F32),
        vm((L, H * Dh), F32),
        vm((SEG, D), F32),
        vm((LANE // L * L, LANE), F32),
        vm((NF, R, 2 * LANE, LANE), F32),
        vm((NF, R, 2 * LANE, LANE), F32),
        pltpu.SemaphoreType.DMA((2 + 4 * ND + 6 + S // 256,)),
    ]
    any_spec = pl.BlockSpec(memory_space=pl.ANY)
    out = pl.pallas_call(
        functools.partial(_kernel, S=S, D=D, H=H, M=M, SEG=SEG, FP=FP),
        out_shape=jax.ShapeDtypeStruct((S, D), BF16),
        in_specs=[any_spec] * 12,
        out_specs=any_spec,
        scratch_shapes=scratch,
        compiler_params=pltpu.CompilerParams(vmem_limit_bytes=110 * 2**20),
    )(A_x.reshape(S, D), A_mem0.reshape(M, D),
      A_Wq.reshape(D * H, Dh), A_Wk.reshape(D * H, Dh), A_Wv.reshape(D * H, Dh),
      A_Wo.reshape(H * Dh, D), B_w_r, B_w_i, *consts)
    return out.reshape(B, S, D)
```

```python
import functools

import jax
import jax.numpy as jnp
import numpy as np
import jax.experimental.pallas as pl
import jax.experimental.pallas.tpu as pltpu

F32, BF16, U32 = jnp.float32, jnp.bfloat16, jnp.uint32
LANE = 128
R = 16


def _dot(a, b):
    return jax.lax.dot_general(a, b, (((1,), (0,)), ((), ())), preferred_element_type=F32)


def _dot_nt(a, b):
    return jax.lax.dot_general(a, b, (((1,), (1,)), ((), ())), preferred_element_type=F32)


def _layernorm(x):
    inv = 1.0 / x.shape[-1]
    c = x - jnp.sum(x, axis=-1, keepdims=True) * inv
    v = jnp.sum(c * c, axis=-1, keepdims=True) * inv
    return c * jax.lax.rsqrt(v + 1e-5)


def _dft_constants(S, D, FP):
    nf = D // 2 + 1
    d = np.arange(D)[:, None]
    k = np.arange(nf)[None, :]
    ang = 2.0 * np.pi * ((d * k) % D) / D
    cos, sin = np.cos(ang), np.sin(ang)
    sin[:, 0] = 0.0
    sin[:, D // 2] = 0.0
    fwd = np.zeros((D, 2 * FP))
    fwd[:, :nf] = cos
    fwd[:, FP:FP + nf] = -sin
    ck = np.full((nf,), 2.0)
    ck[0] = ck[D // 2] = 1.0
    inv = np.zeros((2 * FP, D))
    inv[:nf] = (cos * ck / D).T
    inv[FP:FP + nf] = (-sin * ck / D).T
    k1 = np.arange(R)[:, None, None]
    k2 = np.arange(LANE)[None, :, None]
    n2 = np.arange(LANE)[None, None, :]
    a = 2.0 * np.pi * ((n2 * (k1 + R * k2)) % S) / S
    c, s = np.cos(a), np.sin(a)
    g = np.concatenate([np.concatenate([c, s], 2), np.concatenate([-s, c], 2)], 1)
    gi = np.transpose(g, (0, 2, 1)) / S
    slab = lambda m: np.ascontiguousarray(
        m.reshape(m.shape[0], -1, LANE).transpose(1, 0, 2)).astype(BF16)
    return slab(fwd), slab(inv), g.astype(BF16), gi.astype(BF16)


def _fft4(x, sign):
    (ar, ai), (br, bi), (cr, ci), (dr, di) = x
    sr, si, tr, ti = ar + cr, ai + ci, ar - cr, ai - ci
    ur, ui, vr, vi = br + dr, bi + di, br - dr, bi - di
    p, m = (tr - vi, ti + vr), (tr + vi, ti - vr)
    y1, y3 = (p, m) if sign > 0 else (m, p)
    return [(sr + ur, si + ui), y1, (sr - ur, si - ui), y3]


def _twiddle16(z, e, sign):
    r, i = z
    if e == 0:
        return z
    if e == 4:
        return (-i, r) if sign > 0 else (i, -r)
    c = float(np.cos(2 * np.pi * e / 16))
    s = float(sign * np.sin(2 * np.pi * e / 16))
    if e % 4 == 2:
        sg = s / c
        return ((r - i) * c, (i + r) * c) if sg > 0 else ((r + i) * c, (i - r) * c)
    return (r * c - i * s, i * c + r * s)


def _fft16(x, sign):
    t = [_fft4([x[b + 4 * a] for a in range(4)], sign) for b in range(4)]
    y = [None] * 16
    for k1 in range(4):
        o = _fft4([_twiddle16(t[b][k1], b * k1, sign) for b in range(4)], sign)
        for k2 in range(4):
            y[k1 + 4 * k2] = o[k2]
    return y


def _kernel(x_hbm, mem_hbm, wq_hbm, wk_hbm, wv_hbm, wo_hbm, wr_hbm, wi_hbm,
            fd_hbm, fi_hbm, g_hbm, gi_hbm, out_hbm,
            xb, mem0, stage, wqkv, wo, wrb, wib, wrf, wif, fd, fi, g, gi,
            x, hbuf, oc, otok, fill, xa, ya, bufa, bufb, ob, sems, *, S, D, H, M, SEG, FP):
    L = M + SEG
    nseg = S // SEG
    ND = D // LANE
    NF = FP // LANE
    nf = D // 2 + 1
    G = LANE // L
    groups = [list(range(a, min(a + G, H))) for a in range(0, H, G)]
    scale = LANE ** -0.5
    CH = 256

    rows = LANE * H // 2
    cp_x = pltpu.make_async_copy(x_hbm, xb, sems.at[0])
    cp_mem = pltpu.make_async_copy(mem_hbm, mem0, sems.at[1])
    cp_w = [pltpu.make_async_copy(w.bitcast(U32).at[pl.ds(c * rows, rows)], stage.at[i * ND + c],
                                  sems.at[2 + i * ND + c])
            for i, w in enumerate((wq_hbm, wk_hbm, wv_hbm)) for c in range(ND)]
    n = 2 + 3 * ND
    cp_wo = [pltpu.make_async_copy(wo_hbm.at[:, pl.ds(c * LANE, LANE)], wo.at[c], sems.at[n + c])
             for c in range(ND)]
    n += ND
    cp_b = [pltpu.make_async_copy(a, b, sems.at[n + i]) for i, (a, b) in enumerate(
        ((wr_hbm, wrb), (wi_hbm, wib), (fd_hbm, fd), (fi_hbm, fi), (g_hbm, g), (gi_hbm, gi)))]
    n_out = n + len(cp_b)
    for cp in [cp_x, cp_mem] + cp_w + cp_wo:
        cp.start()

    r = jax.lax.broadcasted_iota(jnp.int32, fill.shape, 0)
    c = jax.lax.broadcasted_iota(jnp.int32, fill.shape, 1)
    rb = sum((r >= L * j).astype(jnp.int32) for j in range(1, G + 1))
    cb = sum((c >= L * j).astype(jnp.int32) for j in range(1, G + 1))
    ri, ci = r - L * rb, c - L * cb
    fill[...] = jnp.where(rb == cb, jnp.where((ri < M) | (ri >= ci), 0.0, -1e9),
                          -jnp.inf).astype(F32)
    otok[...] = jnp.zeros(otok.shape, F32)

    cp_x.wait()

    @pl.loop(0, S // CH)
    def _(i):
        r0 = pl.multiple_of(i * CH, CH)
        x[pl.ds(r0, CH), :] = xb[pl.ds(r0, CH), :].astype(F32)

    cp_mem.wait()

    for t, cp in enumerate(cp_w):
        cp.wait()
        i, c = divmod(t, ND)

        @pl.loop(0, H // 2)
        def _(j):
            w = stage[t, pl.ds(j, LANE, stride=H // 2), :]
            lo = pltpu.bitcast(w << 16, F32).astype(BF16)
            hi = pltpu.bitcast(w & np.uint32(0xFFFF0000), F32).astype(BF16)
            wqkv[i * H + 2 * j, c * LANE:(c + 1) * LANE, :] = lo
            wqkv[i * H + 2 * j + 1, c * LANE:(c + 1) * LANE, :] = hi

    for cp in cp_b:
        cp.start()
    for cp in cp_wo:
        cp.wait()

    def finish_segment(s):
        r0 = pl.multiple_of(s * SEG, SEG)
        xn = x[pl.ds(r0, SEG), :] + otok[...]
        x[pl.ds(r0, SEG), :] = xn
        xb[pl.ds(r0, SEG), :] = _layernorm(xn).astype(BF16)

    def a_step(s, carry):
        st = {}

        def proj(i, hd):
            st[i, hd] = _dot(hbuf[...], wqkv[i * H + hd])

        def scores(gi_):
            gr = groups[gi_]
            pad = [jnp.zeros((LANE - L * len(gr), LANE), F32)]
            q = jnp.concatenate([st.pop((0, hd)) for hd in gr], 0)
            k = jnp.concatenate([st.pop((1, hd)) for hd in gr] + pad, 0).astype(BF16)
            st['v', gi_] = jnp.concatenate([st.pop((2, hd)) for hd in gr] + pad, 0).astype(BF16)
            st['s', gi_] = _dot_nt(q, k)

        def softmax(gi_):
            f = fill[0:L * len(groups[gi_]), :]
            sc = jnp.where(f < 0.0, f, st.pop(('s', gi_)) * scale)
            e = jnp.exp(sc - jnp.max(sc, axis=1, keepdims=True))
            st['p', gi_] = e / jnp.sum(e, axis=1, keepdims=True)

        def values(gi_):
            o = _dot(st.pop(('p', gi_)), st.pop(('v', gi_)))
            for j, hd in enumerate(groups[gi_]):
                oc[:, hd * LANE:(hd + 1) * LANE] = o[L * j:L * (j + 1)]
            done.update(groups[gi_])

        def out_proj(h0, h1):
            a, b = h0 * LANE, h1 * LANE
            t = jnp.concatenate([_dot(oc[:, a:b], wo[c, a:b, :]) for c in range(ND)], 1)
            st['acc'] = st['acc'] + t if 'acc' in st else t

        def next_ln(_):
            r1 = pl.multiple_of(jnp.minimum(s + 1, nseg - 1) * SEG, SEG)
            st['ln'] = _layernorm(x[pl.ds(r1, SEG), :])

        def prev_finish(_):
            finish_segment(jnp.maximum(s - 1, 0))

        events, done = {}, set()
        for gi_, gr in enumerate(groups):
            last = 3 * (gr[-1] + 1) - 1
            for delay, fn in ((0, scores), (3, softmax), (9, values)):
                events.setdefault(last + delay, []).append((fn, gi_))
        events.setdefault(0, []).append((prev_finish, 0))
        events.setdefault(3 * H + 16, []).append((next_ln, 0))
        slot = 0

        def tick():
            nonlocal slot
            for fn, a in events.pop(slot, []):
                fn(a)
            slot += 1

        for gr in groups:
            for i in (1, 0, 2):
                for hd in gr:
                    proj(i, hd)
                    tick()
        WC = 4
        for h0 in range(0, H, WC):
            while not done.issuperset(range(h0, h0 + WC)):
                tick()
            out_proj(h0, h0 + WC)
            for _ in range(WC):
                tick()
        assert not events
        hbuf[M:L, :] = st['ln']
        hbuf[0:M, :] = st['acc'][0:M]
        otok[...] = st['acc'][M:L]
        return carry

    def layer_a():
        hbuf[0:M, :] = mem0[...].astype(F32)
        hbuf[M:L, :] = _layernorm(x[0:SEG, :])
        jax.lax.fori_loop(0, nseg, a_step, 0)
        finish_segment(nseg - 1)
        otok[...] = jnp.zeros(otok.shape, F32)

    RC = 16
    NCH = LANE // RC

    def chunk_rows(i, n1):
        return pl.ds(pl.multiple_of(n1 * LANE + i * RC, RC), RC)

    def dft_fwd(i, buf):
        xh = jnp.concatenate([xb[chunk_rows(i, n1), :] for n1 in range(R)], 0)
        for c in range(2 * NF):
            buf[c] = _dot(xh, fd[c])
            yield

    def radix_fwd(i, buf):
        for c in range(NF):
            for h in range(0, RC, 8):
                v = [(buf[c, n1 * RC + h:n1 * RC + h + 8, :],
                      buf[NF + c, n1 * RC + h:n1 * RC + h + 8, :]) for n1 in range(R)]
                r0 = pl.multiple_of(i * RC + h, 8)
                for k1, (re, im) in enumerate(_fft16(v, -1)):
                    ya[c, k1, pl.ds(r0, 8), :] = re
                    ya[c, k1, pl.ds(LANE + r0, 8), :] = im
                yield

    def filter_transpose(i):
        n_ = S // NCH
        cols = pl.ds(pl.multiple_of(i * n_, n_), n_)
        for src, dst in ((wrb, wrf), (wib, wif)):
            for c in range(NF):
                lo, hi = c * LANE, min((c + 1) * LANE, nf)
                t = src[lo:hi, cols].astype(F32)
                if hi - lo < LANE:
                    t = jnp.concatenate([t, jnp.zeros((LANE - (hi - lo), n_), F32)], 0)
                dst[c, cols, :] = t.T
                yield

    def radix_inv(i, buf):
        for c in range(NF):
            for h in range(0, RC, 8):
                r0 = pl.multiple_of(i * RC + h, 8)
                v = [(xa[c, k1, pl.ds(r0, 8), :], xa[c, k1, pl.ds(LANE + r0, 8), :])
                     for k1 in range(R)]
                for n1, (re, im) in enumerate(_fft16(v, +1)):
                    buf[c, n1 * RC + h:n1 * RC + h + 8, :] = re
                    buf[NF + c, n1 * RC + h:n1 * RC + h + 8, :] = im
                yield

    def out_copy(i):
        rs = pl.ds(pl.multiple_of(i * RC, RC), RC)
        return pltpu.make_async_copy(ob.at[:, rs, :], out_hbm.at[:, rs, :], sems.at[n_out + i])

    def dft_inv(i, buf):
        zz = jnp.concatenate([buf[c] for c in range(2 * NF)], 1).astype(BF16)
        for c in range(ND):
            y = _dot(zz, fi[c])
            cs = slice(c * LANE, (c + 1) * LANE)
            for n1 in range(R):
                xn = x[chunk_rows(i, n1), cs] + y[n1 * RC:(n1 + 1) * RC]
                x[chunk_rows(i, n1), cs] = xn
                ob[n1, pl.ds(pl.multiple_of(i * RC, RC), RC), cs] = xn.astype(BF16)
            yield

    def interleave(*gens):
        gens = list(gens)
        while gens:
            gens = [gen for gen in gens if next(gen, False) is None]

    def layer_b(layer):
        interleave(dft_fwd(0, bufa))

        @pl.loop(0, NCH // 2 - 1)
        def _(j):
            interleave(dft_fwd(2 * j + 1, bufb), radix_fwd(2 * j, bufa), filter_transpose(2 * j))
            interleave(dft_fwd(2 * j + 2, bufa), radix_fwd(2 * j + 1, bufb),
                       filter_transpose(2 * j + 1))

        interleave(dft_fwd(NCH - 1, bufb), radix_fwd(NCH - 2, bufa),
                   filter_transpose(NCH - 2), filter_transpose(NCH - 1))
        interleave(radix_fwd(NCH - 1, bufb))
        U = 4

        @pl.loop(0, R // U)
        def _(j):
            items = [(j * U + u, c) for u in range(U) for c in range(NF)]
            z = {}
            for t in range(len(items) + 2):
                if t < len(items):
                    k1, c = items[t]
                    z[t] = _dot(g[k1], ya[c, k1].astype(BF16))
                if t >= 2:
                    k1, c = items[t - 2]
                    zt = z.pop(t - 2)
                    zr, zi = zt[0:LANE], zt[LANE:]
                    wr = wrf[c, pl.ds(k1, LANE, stride=R), :]
                    wi = wif[c, pl.ds(k1, LANE, stride=R), :]
                    zz = jnp.concatenate([zr * wr - zi * wi, zr * wi + zi * wr], 0)
                    xa[c, k1] = _dot(gi[k1], zz.astype(BF16))

        def send(i):
            @pl.when(layer == 1)
            def _():
                out_copy(i).start()

        interleave(radix_inv(0, bufa))

        @pl.loop(0, NCH // 2 - 1)
        def _(j):
            interleave(dft_inv(2 * j, bufa), radix_inv(2 * j + 1, bufb))
            interleave(dft_inv(2 * j + 1, bufb), radix_inv(2 * j + 2, bufa))
            send(2 * j)
            send(2 * j + 1)

        interleave(dft_inv(NCH - 2, bufa), radix_inv(NCH - 1, bufb))
        interleave(dft_inv(NCH - 1, bufb))
        send(NCH - 2)
        send(NCH - 1)

    @pl.loop(0, 2)
    def _(layer):
        layer_a()

        @pl.when(layer == 0)
        def _():
            for cp in cp_b:
                cp.wait()

        layer_b(layer)

    for i in range(NCH):
        out_copy(i).wait()


@functools.partial(jax.jit, static_argnames=("A_seg_len",))
def pallas_interleave_layers__memory_aug_recurrent_mem_tr__spectral_gfnet__prompt_kernel(
    A_x, A_mem0, A_Wq, A_Wk, A_Wv, A_Wo, A_seg_len, B_x, B_w_r, B_w_i,
):
    del B_x
    B, S, D = A_x.shape
    _, H, Dh = A_Wq.shape
    M = A_mem0.shape[1]
    SEG = int(A_seg_len)
    nf = D // 2 + 1
    FP = -(-nf // LANE) * LANE
    L = M + SEG
    assert B == 1 and Dh == LANE and S == R * LANE and D % LANE == 0 and S % SEG == 0
    assert M % 8 == 0 and SEG % 16 == 0 and L <= LANE and H % 4 == 0
    ND, NF = D // LANE, FP // LANE
    consts = _dft_constants(S, D, FP)

    vm = pltpu.VMEM
    scratch = [
        vm((S, D), BF16),
        vm((M, D), BF16),
        vm((3 * ND, LANE * H // 2, LANE), U32),
        vm((3 * H, D, LANE), BF16),
        vm((ND, H * Dh, LANE), BF16),
        vm((nf, S), BF16), vm((nf, S), BF16),
        vm((NF, S, LANE), F32), vm((NF, S, LANE), F32),
        vm(consts[0].shape, BF16), vm(consts[1].shape, BF16),
        vm(consts[2].shape, BF16), vm(consts[3].shape, BF16),
        vm((S, D), F32),
        vm((L, D), F32),
        vm((L, H * Dh), F32),
        vm((SEG, D), F32),
        vm((LANE // L * L, LANE), F32),
        vm((NF, R, 2 * LANE, LANE), F32),
        vm((NF, R, 2 * LANE, LANE), F32),
        vm((2 * NF, R * 16, LANE), F32),
        vm((2 * NF, R * 16, LANE), F32),
        vm((R, LANE, D), BF16),
        pltpu.SemaphoreType.DMA((2 + 4 * ND + 6 + LANE // 16,)),
    ]
    any_spec = pl.BlockSpec(memory_space=pltpu.HBM)
    out = pl.pallas_call(
        functools.partial(_kernel, S=S, D=D, H=H, M=M, SEG=SEG, FP=FP),
        out_shape=jax.ShapeDtypeStruct((R, LANE, D), BF16),
        in_specs=[any_spec] * 12,
        out_specs=any_spec,
        scratch_shapes=scratch,
        compiler_params=pltpu.CompilerParams(vmem_limit_bytes=110 * 2**20),
    )(A_x.reshape(S, D), A_mem0.reshape(M, D),
      A_Wq.reshape(D * H, Dh), A_Wk.reshape(D * H, Dh), A_Wv.reshape(D * H, Dh),
      A_Wo.reshape(H * Dh, D), B_w_r.T, B_w_i.T, *consts)
    return out.reshape(B, S, D)
```

```python
import functools

import jax
import jax.numpy as jnp
import numpy as np
import jax.experimental.pallas as pl
import jax.experimental.pallas.tpu as pltpu

F32, BF16, U32 = jnp.float32, jnp.bfloat16, jnp.uint32
LANE = 128
R = 16


def _dot(a, b):
    return jax.lax.dot_general(a, b, (((1,), (0,)), ((), ())), preferred_element_type=F32)


def _dot_nt(a, b):
    return jax.lax.dot_general(a, b, (((1,), (1,)), ((), ())), preferred_element_type=F32)


def _layernorm(x):
    inv = 1.0 / x.shape[-1]
    c = x - jnp.sum(x, axis=-1, keepdims=True) * inv
    v = jnp.sum(c * c, axis=-1, keepdims=True) * inv
    return c * jax.lax.rsqrt(v + 1e-5)


def _after(w, token):
    if token is None:
        return w
    head = pltpu.bitcast(pltpu.bitcast(w[0:16], U32) | token, BF16)
    return jnp.concatenate([head, w[16:]], 0)


def _dft_constants(S, D, FP):
    nf = D // 2 + 1
    d = np.arange(D)[:, None]
    k = np.arange(nf)[None, :]
    ang = 2.0 * np.pi * ((d * k) % D) / D
    cos, sin = np.cos(ang), np.sin(ang)
    n0 = FP - LANE
    ck = np.full((nf,), 2.0)
    ck[0] = ck[D // 2] = 1.0

    def pack(re, im):
        return np.concatenate(
            [re[:, :n0], re[:, D // 2:], im[:, 1:n0], re[:, n0:D // 2], im[:, n0:D // 2]], 1)

    fwd = pack(cos, -sin)
    inv = pack(cos * ck / D, -sin * ck / D).T
    k1 = np.arange(R)[:, None, None]
    k2 = np.arange(LANE)[None, :, None]
    n2 = np.arange(LANE)[None, None, :]
    a = 2.0 * np.pi * ((n2 * (k1 + R * k2)) % S) / S
    c, s = np.cos(a), np.sin(a)
    g = np.concatenate([np.concatenate([c, s], 2), np.concatenate([-s, c], 2)], 1)
    gi = np.transpose(g, (0, 2, 1)) / S
    slab = lambda m: np.ascontiguousarray(
        m.reshape(m.shape[0], -1, LANE).transpose(1, 0, 2)).astype(BF16)
    return slab(fwd), slab(inv), g.astype(BF16), gi.astype(BF16)


def _fft4(x, sign):
    (ar, ai), (br, bi), (cr, ci), (dr, di) = x
    sr, si, tr, ti = ar + cr, ai + ci, ar - cr, ai - ci
    ur, ui, vr, vi = br + dr, bi + di, br - dr, bi - di
    p, m = (tr - vi, ti + vr), (tr + vi, ti - vr)
    y1, y3 = (p, m) if sign > 0 else (m, p)
    return [(sr + ur, si + ui), y1, (sr - ur, si - ui), y3]


def _twiddle16(z, e, sign):
    r, i = z
    if e == 0:
        return z
    if e == 4:
        return (-i, r) if sign > 0 else (i, -r)
    c = float(np.cos(2 * np.pi * e / 16))
    s = float(sign * np.sin(2 * np.pi * e / 16))
    if e % 4 == 2:
        sg = s / c
        return ((r - i) * c, (i + r) * c) if sg > 0 else ((r + i) * c, (i - r) * c)
    return (r * c - i * s, i * c + r * s)


def _fft16(x, sign):
    t = [_fft4([x[b + 4 * a] for a in range(4)], sign) for b in range(4)]
    y = [None] * 16
    for k1 in range(4):
        o = _fft4([_twiddle16(t[b][k1], b * k1, sign) for b in range(4)], sign)
        for k2 in range(4):
            y[k1 + 4 * k2] = o[k2]
    return y


def _kernel(x_hbm, mem_hbm, wq_hbm, wk_hbm, wv_hbm, wo_hbm, wr_hbm, wi_hbm,
            fd_hbm, fi_hbm, g_hbm, gi_hbm, out_hbm,
            xb, mem0, stage, wqkv, wo, wrb, wib, wrf, wif, fd, fi, g, gi,
            x, hbuf, oc, otok, fill, xa, ya, bufa, bufb, ob, sems, *, S, D, H, M, SEG, FP):
    L = M + SEG
    nseg = S // SEG
    ND = D // LANE
    NF = FP // LANE
    nf = D // 2 + 1
    G = LANE // L
    groups = [list(range(a, min(a + G, H))) for a in range(0, H, G)]
    scale = LANE ** -0.5
    CH = 256

    rows = LANE * H // 2
    cp_x = pltpu.make_async_copy(x_hbm, xb, sems.at[0])
    cp_mem = pltpu.make_async_copy(mem_hbm, mem0, sems.at[1])
    cp_w = [pltpu.make_async_copy(w.bitcast(U32).at[pl.ds(c * rows, rows)], stage.at[i * ND + c],
                                  sems.at[2 + i * ND + c])
            for i, w in enumerate((wq_hbm, wk_hbm, wv_hbm)) for c in range(ND)]
    n = 2 + 3 * ND
    cp_wo = [pltpu.make_async_copy(wo_hbm.at[:, pl.ds(c * LANE, LANE)], wo.at[c], sems.at[n + c])
             for c in range(ND)]
    n += ND
    cp_b = [pltpu.make_async_copy(a, b, sems.at[n + i]) for i, (a, b) in enumerate(
        ((wr_hbm, wrb), (wi_hbm, wib), (fd_hbm, fd), (fi_hbm, fi), (g_hbm, g), (gi_hbm, gi)))]
    n_out = n + len(cp_b)
    for cp in [cp_x, cp_mem] + cp_w + cp_wo:
        cp.start()

    r = jax.lax.broadcasted_iota(jnp.int32, fill.shape, 0)
    c = jax.lax.broadcasted_iota(jnp.int32, fill.shape, 1)
    rb = sum((r >= L * j).astype(jnp.int32) for j in range(1, G + 1))
    cb = sum((c >= L * j).astype(jnp.int32) for j in range(1, G + 1))
    ri, ci = r - L * rb, c - L * cb
    fill[...] = jnp.where(rb == cb, jnp.where((ri < M) | (ri >= ci), 0.0, -1e9),
                          -jnp.inf).astype(F32)
    otok[...] = jnp.zeros(otok.shape, F32)

    cp_x.wait()

    @pl.loop(0, S // CH)
    def _(i):
        r0 = pl.multiple_of(i * CH, CH)
        x[pl.ds(r0, CH), :] = xb[pl.ds(r0, CH), :].astype(F32)

    cp_mem.wait()

    for t, cp in enumerate(cp_w):
        cp.wait()
        i, c = divmod(t, ND)

        @pl.loop(0, H // 2)
        def _(j):
            w = stage[t, pl.ds(j, LANE, stride=H // 2), :]
            lo = pltpu.bitcast(w << 16, F32).astype(BF16)
            hi = pltpu.bitcast(w & np.uint32(0xFFFF0000), F32).astype(BF16)
            wqkv[i * H + 2 * j, c * LANE:(c + 1) * LANE, :] = lo
            wqkv[i * H + 2 * j + 1, c * LANE:(c + 1) * LANE, :] = hi

    for cp in cp_b:
        cp.start()
    for cp in cp_wo:
        cp.wait()

    def token(zero, *vals):
        bits = functools.reduce(jnp.bitwise_or, [pltpu.bitcast(v, U32) for v in vals])
        return bits & zero.astype(U32)

    def finish_segment(s):
        r0 = pl.multiple_of(s * SEG, SEG)
        xn = x[pl.ds(r0, SEG), :] + otok[...]
        x[pl.ds(r0, SEG), :] = xn
        ln = _layernorm(xn)
        xb[pl.ds(r0, SEG), :] = ln.astype(BF16)
        return ln

    def a_step(s, carry):
        st = {}

        def proj(i, hd):
            st[i, hd] = _dot(hbuf[...], _after(wqkv[i * H + hd], st.pop(('tok', slot), None)))

        def scores(gi_):
            gr = groups[gi_]
            pad = [jnp.zeros((LANE - L * len(gr), LANE), F32)]
            q = jnp.concatenate([st.pop((0, hd)) for hd in gr], 0)
            k = jnp.concatenate([st.pop((1, hd)) for hd in gr] + pad, 0).astype(BF16)
            st['v', gi_] = jnp.concatenate([st.pop((2, hd)) for hd in gr] + pad, 0).astype(BF16)
            st['s', gi_] = _dot_nt(q, k)

        def softmax(gi_):
            f = fill[0:L * len(groups[gi_]), :]
            sc = jnp.where(f < 0.0, f, st.pop(('s', gi_)) * scale)
            e = jnp.exp(sc - jnp.max(sc, axis=1, keepdims=True))
            st['p', gi_] = e / jnp.sum(e, axis=1, keepdims=True)

        def values(gi_):
            o = _dot(st.pop(('p', gi_)), st.pop(('v', gi_)))
            for j, hd in enumerate(groups[gi_]):
                oc[:, hd * LANE:(hd + 1) * LANE] = o[L * j:L * (j + 1)]
            done.update(groups[gi_])

        def out_proj(h0, h1):
            a, b = h0 * LANE, h1 * LANE
            tok = st.pop(('tok', slot), None)
            t = jnp.concatenate(
                [_dot(oc[:, a:b], _after(wo[c, a:b, :], tok if c == 0 else None))
                 for c in range(ND)], 1)
            st['acc'] = st['acc'] + t if 'acc' in st else t

        def next_ln(_):
            r1 = pl.multiple_of(jnp.minimum(s + 1, nseg - 1) * SEG, SEG)
            ln = _layernorm(x[pl.ds(r1, SEG), :])
            hbuf[M:L, :] = ln
            st['tok', 3 * H + 24] = token(
                s >> 16, *[ln[a:a + 8, D - LANE:] for a in range(0, SEG, 8)])

        def prev_finish(_):
            ln = finish_segment(jnp.maximum(s - 1, 0))
            st['tok', 11] = token(s >> 16, *[ln[a:a + 8, D - LANE:] for a in range(0, SEG, 8)])

        events, done = {}, set()
        for gi_, gr in enumerate(groups):
            last = 3 * (gr[-1] + 1) - 1
            for delay, fn in ((0, scores), (3, softmax), (9, values)):
                events.setdefault(last + delay, []).append((fn, gi_))
        events.setdefault(0, []).append((prev_finish, 0))
        events.setdefault(3 * H + 16, []).append((next_ln, 0))
        slot = 0

        def tick():
            nonlocal slot
            for fn, a in events.pop(slot, []):
                fn(a)
            slot += 1

        for gr in groups:
            for i in (1, 0, 2):
                for hd in gr:
                    proj(i, hd)
                    tick()
        WC = 4
        for h0 in range(0, H, WC):
            while not done.issuperset(range(h0, h0 + WC)):
                tick()
            out_proj(h0, h0 + WC)
            for _ in range(WC):
                tick()
        assert not events and set(st) == {'acc'}
        hbuf[0:M, :] = st['acc'][0:M]
        otok[...] = st['acc'][M:L]
        return carry

    def layer_a():
        hbuf[0:M, :] = mem0[...].astype(F32)
        hbuf[M:L, :] = _layernorm(x[0:SEG, :])
        jax.lax.fori_loop(0, nseg, a_step, 0)
        finish_segment(nseg - 1)
        otok[...] = jnp.zeros(otok.shape, F32)

    RC = 16
    NCH = LANE // RC

    def chunk_rows(i, n1):
        return pl.ds(pl.multiple_of(n1 * LANE + i * RC, RC), RC)

    lane = jax.lax.broadcasted_iota(jnp.int32, (8, LANE), 1)
    HALF = LANE // 2
    IM0, MIX = NF - 1, 2 * NF - 2

    def dft_fwd(i, buf):
        xh = jnp.concatenate([xb[chunk_rows(i, n1), :] for n1 in range(R)], 0)
        for c in [c_ + o for c_ in range(NF - 1) for o in (0, IM0)] + [MIX]:
            buf[c] = _dot(xh, _after(fd[c], (yield)))

    def radix_fwd(i, buf, zero):
        for c in range(NF):
            for h in range(0, RC, 8):
                def load(n1):
                    rs = slice(n1 * RC + h, n1 * RC + h + 8)
                    if c < NF - 1:
                        im = buf[IM0 + c, rs, :]
                        return buf[c, rs, :], jnp.where(lane == 0, 0.0, im) if c == 0 else im
                    t = buf[MIX, rs, :]
                    u = pltpu.roll(jnp.where(lane == 0, buf[IM0, rs, :], t), HALF, 1)
                    return jnp.where(lane == HALF, u, t), jnp.where(lane == HALF, 0.0, u)

                r0 = pl.multiple_of(i * RC + h, 8)
                for k1, (re, im) in enumerate(_fft16([load(n1) for n1 in range(R)], -1)):
                    ya[c, k1, pl.ds(r0, 8), :] = re
                    ya[c, k1, pl.ds(LANE + r0, 8), :] = im
            yield ya[c, 0, pl.ds(pl.multiple_of(i * RC + zero, 8), 8), :]

    def filter_transpose(i):
        n_ = S // NCH
        cols = pl.ds(pl.multiple_of(i * n_, n_), n_)
        for c in range(NF):
            for src, dst in ((wrb, wrf), (wib, wif)):
                lo, hi = c * LANE, min((c + 1) * LANE, nf)
                t = src[lo:hi, cols].astype(F32)
                if hi - lo < LANE:
                    t = jnp.concatenate([t, jnp.zeros((LANE - (hi - lo), n_), F32)], 0)
                t = t.T
                dst[c, cols, :] = t
            yield t[n_ - 8:]

    def radix_inv(i, buf, zero):
        for c in range(NF):
            for h in range(0, RC, 8):
                r0 = pl.multiple_of(i * RC + h, 8)
                v = [(xa[c, k1, pl.ds(r0, 8), :], xa[c, k1, pl.ds(LANE + r0, 8), :])
                     for k1 in range(R)]
                for n1, (re, im) in enumerate(_fft16(v, +1)):
                    rs = slice(n1 * RC + h, n1 * RC + h + 8)
                    if c < NF - 1:
                        buf[c, rs, :] = re
                        buf[IM0 + c, rs, :] = im
                    else:
                        u = pltpu.roll(jnp.where(lane == HALF, re, im), HALF, 1)
                        buf[MIX, rs, :] = jnp.where(lane < HALF, re, u)
                        buf[IM0, rs, :] = jnp.where(lane == 0, u, buf[IM0, rs, :])
            yield buf[0, pl.ds(pl.multiple_of(zero, 8), 8), :]

    def out_copy(i):
        rs = pl.ds(pl.multiple_of(i * RC, RC), RC)
        return pltpu.make_async_copy(ob.at[:, rs, :], out_hbm.at[:, rs, :], sems.at[n_out + i])

    def dft_inv(i, buf, zero):
        zz = jnp.concatenate([buf[c] for c in range(ND)], 1).astype(BF16)
        for c in range(ND):
            y = _dot(zz, _after(fi[c], (yield)))
            cs = slice(c * LANE, (c + 1) * LANE)
            for n1 in range(R):
                xn = x[chunk_rows(i, n1), cs] + y[n1 * RC:(n1 + 1) * RC]
                x[chunk_rows(i, n1), cs] = xn
                ob[n1, pl.ds(pl.multiple_of(i * RC, RC), RC), cs] = xn.astype(BF16)

    def overlap(zero, mxu, *vpu):
        LAG = 2
        next(mxu)
        toks = [None] * LAG
        while True:
            vals = [v for v in (next(gen, None) for gen in vpu) if v is not None]
            toks.append(token(zero, *vals) if vals else None)
            try:
                mxu.send(toks.pop(0))
            except StopIteration:
                break

    def layer_b(layer):
        zero = layer >> 8
        overlap(zero, dft_fwd(0, bufa), filter_transpose(0))

        @pl.loop(0, NCH // 2 - 1)
        def _(j):
            overlap(zero, dft_fwd(2 * j + 1, bufb), radix_fwd(2 * j, bufa, zero),
                    filter_transpose(2 * j + 1))
            overlap(zero, dft_fwd(2 * j + 2, bufa), radix_fwd(2 * j + 1, bufb, zero),
                    filter_transpose(2 * j + 2))

        overlap(zero, dft_fwd(NCH - 1, bufb), radix_fwd(NCH - 2, bufa, zero),
                filter_transpose(NCH - 1))
        list(radix_fwd(NCH - 1, bufb, zero))
        U = 4

        @pl.loop(0, R // U)
        def _(j):
            items = [(j * U + u, c) for u in range(U) for c in range(NF)]
            z = {}
            for t in range(len(items) + 2):
                if t < len(items):
                    k1, c = items[t]
                    z[t] = _dot(g[k1], ya[c, k1].astype(BF16))
                if t >= 2:
                    k1, c = items[t - 2]
                    zt = z.pop(t - 2)
                    zr, zi = zt[0:LANE], zt[LANE:]
                    wr = wrf[c, pl.ds(k1, LANE, stride=R), :]
                    wi = wif[c, pl.ds(k1, LANE, stride=R), :]
                    zz = jnp.concatenate([zr * wr - zi * wi, zr * wi + zi * wr], 0)
                    xa[c, k1] = _dot(gi[k1], zz.astype(BF16))

        def send(i):
            @pl.when(layer == 1)
            def _():
                out_copy(i).start()

        list(radix_inv(0, bufa, zero))

        @pl.loop(0, NCH // 2 - 1)
        def _(j):
            overlap(zero, dft_inv(2 * j, bufa, zero), radix_inv(2 * j + 1, bufb, zero))
            overlap(zero, dft_inv(2 * j + 1, bufb, zero), radix_inv(2 * j + 2, bufa, zero))
            send(2 * j)
            send(2 * j + 1)

        overlap(zero, dft_inv(NCH - 2, bufa, zero), radix_inv(NCH - 1, bufb, zero))
        overlap(zero, dft_inv(NCH - 1, bufb, zero))
        send(NCH - 2)
        send(NCH - 1)

    @pl.loop(0, 2)
    def _(layer):
        layer_a()

        @pl.when(layer == 0)
        def _():
            for cp in cp_b:
                cp.wait()

        layer_b(layer)

    for i in range(NCH):
        out_copy(i).wait()


@functools.partial(jax.jit, static_argnames=("A_seg_len",))
def pallas_interleave_layers__memory_aug_recurrent_mem_tr__spectral_gfnet__prompt_kernel(
    A_x, A_mem0, A_Wq, A_Wk, A_Wv, A_Wo, A_seg_len, B_x, B_w_r, B_w_i,
):
    del B_x
    B, S, D = A_x.shape
    _, H, Dh = A_Wq.shape
    M = A_mem0.shape[1]
    SEG = int(A_seg_len)
    nf = D // 2 + 1
    FP = -(-nf // LANE) * LANE
    L = M + SEG
    assert B == 1 and Dh == LANE and S == R * LANE and D % LANE == 0 and S % SEG == 0
    assert M % 8 == 0 and SEG % 16 == 0 and L <= LANE and H % 4 == 0 and D // LANE % 2 == 1
    ND, NF = D // LANE, FP // LANE
    consts = _dft_constants(S, D, FP)

    vm = pltpu.VMEM
    scratch = [
        vm((S, D), BF16),
        vm((M, D), BF16),
        vm((3 * ND, LANE * H // 2, LANE), U32),
        vm((3 * H, D, LANE), BF16),
        vm((ND, H * Dh, LANE), BF16),
        vm((nf, S), BF16), vm((nf, S), BF16),
        vm((NF, S, LANE), F32), vm((NF, S, LANE), F32),
        vm(consts[0].shape, BF16), vm(consts[1].shape, BF16),
        vm(consts[2].shape, BF16), vm(consts[3].shape, BF16),
        vm((S, D), F32),
        vm((L, D), F32),
        vm((L, H * Dh), F32),
        vm((SEG, D), F32),
        vm((LANE // L * L, LANE), F32),
        vm((NF, R, 2 * LANE, LANE), F32),
        vm((NF, R, 2 * LANE, LANE), F32),
        vm((ND, R * 16, LANE), F32),
        vm((ND, R * 16, LANE), F32),
        vm((R, LANE, D), BF16),
        pltpu.SemaphoreType.DMA((2 + 4 * ND + 6 + LANE // 16,)),
    ]
    any_spec = pl.BlockSpec(memory_space=pltpu.HBM)
    out = pl.pallas_call(
        functools.partial(_kernel, S=S, D=D, H=H, M=M, SEG=SEG, FP=FP),
        out_shape=jax.ShapeDtypeStruct((R, LANE, D), BF16),
        in_specs=[any_spec] * 12,
        out_specs=any_spec,
        scratch_shapes=scratch,
        compiler_params=pltpu.CompilerParams(vmem_limit_bytes=110 * 2**20),
    )(A_x.reshape(S, D), A_mem0.reshape(M, D),
      A_Wq.reshape(D * H, Dh), A_Wk.reshape(D * H, Dh), A_Wv.reshape(D * H, Dh),
      A_Wo.reshape(H * Dh, D), B_w_r.T, B_w_i.T, *consts)
    return out.reshape(B, S, D)
```

```python
import functools

import jax
import jax.numpy as jnp
import numpy as np
import jax.experimental.pallas as pl
import jax.experimental.pallas.tpu as pltpu

F32, BF16, U32 = jnp.float32, jnp.bfloat16, jnp.uint32
LANE = 128
R = 16


def _dot(a, b):
    return jax.lax.dot_general(a, b, (((1,), (0,)), ((), ())), preferred_element_type=F32)


def _dot_nt(a, b):
    return jax.lax.dot_general(a, b, (((1,), (1,)), ((), ())), preferred_element_type=F32)


def _layernorm(x):
    inv = 1.0 / x.shape[-1]
    c = x - jnp.sum(x, axis=-1, keepdims=True) * inv
    v = jnp.sum(c * c, axis=-1, keepdims=True) * inv
    return c * jax.lax.rsqrt(v + 1e-5)


def _after(w, token):
    if token is None:
        return w
    head = pltpu.bitcast(pltpu.bitcast(w[0:16], U32) | token, BF16)
    return jnp.concatenate([head, w[16:]], 0)


def _dft_constants(S, D, FP):
    nf = D // 2 + 1
    d = np.arange(D)[:, None]
    k = np.arange(nf)[None, :]
    ang = 2.0 * np.pi * ((d * k) % D) / D
    cos, sin = np.cos(ang), np.sin(ang)
    n0 = FP - LANE
    ck = np.full((nf,), 2.0)
    ck[0] = ck[D // 2] = 1.0

    def pack(re, im):
        return np.concatenate(
            [re[:, :n0], re[:, D // 2:], im[:, 1:n0], re[:, n0:D // 2], im[:, n0:D // 2]], 1)

    fwd = pack(cos, -sin)
    inv = pack(cos * ck / D, -sin * ck / D).T
    k1 = np.arange(R)[:, None, None]
    k2 = np.arange(LANE)[None, :, None]
    n2 = np.arange(LANE)[None, None, :]
    a = 2.0 * np.pi * ((n2 * (k1 + R * k2)) % S) / S
    c, s = np.cos(a), np.sin(a)
    g = np.concatenate([np.concatenate([c, s], 2), np.concatenate([-s, c], 2)], 1)
    gi = np.transpose(g, (0, 2, 1)) / S
    slab = lambda m: np.ascontiguousarray(
        m.reshape(m.shape[0], -1, LANE).transpose(1, 0, 2)).astype(BF16)
    return slab(fwd), slab(inv), g.astype(BF16), gi.astype(BF16)


def _fft4(x, sign):
    (ar, ai), (br, bi), (cr, ci), (dr, di) = x
    sr, si, tr, ti = ar + cr, ai + ci, ar - cr, ai - ci
    ur, ui, vr, vi = br + dr, bi + di, br - dr, bi - di
    p, m = (tr - vi, ti + vr), (tr + vi, ti - vr)
    y1, y3 = (p, m) if sign > 0 else (m, p)
    return [(sr + ur, si + ui), y1, (sr - ur, si - ui), y3]


def _twiddle16(z, e, sign):
    r, i = z
    if e == 0:
        return z
    if e == 4:
        return (-i, r) if sign > 0 else (i, -r)
    c = float(np.cos(2 * np.pi * e / 16))
    s = float(sign * np.sin(2 * np.pi * e / 16))
    if e % 4 == 2:
        sg = s / c
        return ((r - i) * c, (i + r) * c) if sg > 0 else ((r + i) * c, (i - r) * c)
    return (r * c - i * s, i * c + r * s)


def _fft16(x, sign):
    t = [_fft4([x[b + 4 * a] for a in range(4)], sign) for b in range(4)]
    y = [None] * 16
    for k1 in range(4):
        o = _fft4([_twiddle16(t[b][k1], b * k1, sign) for b in range(4)], sign)
        for k2 in range(4):
            y[k1 + 4 * k2] = o[k2]
    return y


def _kernel(x_hbm, mem_hbm, wq_hbm, wk_hbm, wv_hbm, wo_hbm, wr_hbm, wi_hbm,
            fd_hbm, fi_hbm, g_hbm, gi_hbm, out_hbm,
            xin, xb, mem0, stage, wqkv, wo, wrb, wib, wrf, wif, fd, fi, g, gi,
            x, hbuf, oc, otok, fill, xa, ya, bufa, bufb, ob, sems, *, S, D, H, M, SEG, FP):
    L = M + SEG
    nseg = S // SEG
    ND = D // LANE
    NF = FP // LANE
    nf = D // 2 + 1
    G = LANE // L
    groups = [list(range(a, min(a + G, H))) for a in range(0, H, G)]
    scale = LANE ** -0.5
    UA = 2
    CH = 2 * UA * SEG

    rows = LANE * H // 2
    cp_x = pltpu.make_async_copy(x_hbm.at[0:CH], xb.at[0:CH], sems.at[0])
    cp_x2 = pltpu.make_async_copy(x_hbm.at[CH:S], xin.at[CH:S], sems.at[0])
    cp_mem = pltpu.make_async_copy(mem_hbm, mem0, sems.at[1])
    cp_w = [pltpu.make_async_copy(w.bitcast(U32).at[pl.ds(c * rows, rows)], stage.at[i * ND + c],
                                  sems.at[2 + i * ND + c])
            for i, w in enumerate((wq_hbm, wk_hbm, wv_hbm)) for c in range(ND)]
    n = 2 + 3 * ND
    cp_wo = [pltpu.make_async_copy(wo_hbm.at[:, pl.ds(c * LANE, LANE)], wo.at[c], sems.at[n + c])
             for c in range(ND)]
    n += ND
    cp_b = [pltpu.make_async_copy(a, b, sems.at[n + i]) for i, (a, b) in enumerate(
        ((wr_hbm, wrb), (wi_hbm, wib), (fd_hbm, fd), (fi_hbm, fi), (g_hbm, g), (gi_hbm, gi)))]
    n_out = n + len(cp_b)
    queue = cp_w + cp_wo
    DEPTH = 4
    for cp in [cp_x, cp_mem] + queue[:DEPTH]:
        cp.start()

    r = jax.lax.broadcasted_iota(jnp.int32, fill.shape, 0)
    c = jax.lax.broadcasted_iota(jnp.int32, fill.shape, 1)
    rb = sum((r >= L * j).astype(jnp.int32) for j in range(1, G + 1))
    cb = sum((c >= L * j).astype(jnp.int32) for j in range(1, G + 1))
    ri, ci = r - L * rb, c - L * cb
    fill[...] = jnp.where(rb == cb, jnp.where((ri < M) | (ri >= ci), 0.0, -1e9),
                          -jnp.inf).astype(F32)
    otok[...] = jnp.zeros(otok.shape, F32)

    cp_x.wait()
    x[0:CH, :] = xb[0:CH, :].astype(F32)
    cp_mem.wait()

    for t, cp in enumerate(cp_w):
        cp.wait()
        queue[t + DEPTH].start()
        i, c = divmod(t, ND)

        @pl.loop(0, H // 2)
        def _(j):
            w = stage[t, pl.ds(j, LANE, stride=H // 2), :]
            lo = pltpu.bitcast(w << 16, F32).astype(BF16)
            hi = pltpu.bitcast(w & np.uint32(0xFFFF0000), F32).astype(BF16)
            wqkv[i * H + 2 * j, c * LANE:(c + 1) * LANE, :] = lo
            wqkv[i * H + 2 * j + 1, c * LANE:(c + 1) * LANE, :] = hi

    for cp in queue[len(cp_w) + DEPTH:]:
        cp.start()
    for cp in cp_wo:
        cp.wait()
    cp_x2.start()

    def token(zero, *vals):
        bits = functools.reduce(jnp.bitwise_or, [pltpu.bitcast(v, U32) for v in vals])
        return bits & zero.astype(U32)

    def finish_segment(s):
        r0 = pl.multiple_of(s * SEG, SEG)
        xn = x[pl.ds(r0, SEG), :] + otok[...]
        x[pl.ds(r0, SEG), :] = xn
        ln = _layernorm(xn)
        xb[pl.ds(r0, SEG), :] = ln.astype(BF16)
        return ln

    def a_step(s):
        st = {}

        def proj(i, hd):
            st[i, hd] = _dot(hbuf[...], _after(wqkv[i * H + hd], st.pop(('tok', slot), None)))

        def scores(gi_):
            gr = groups[gi_]
            pad = [jnp.zeros((LANE - L * len(gr), LANE), F32)]
            q = jnp.concatenate([st.pop((0, hd)) for hd in gr], 0)
            k = jnp.concatenate([st.pop((1, hd)) for hd in gr] + pad, 0).astype(BF16)
            st['v', gi_] = jnp.concatenate([st.pop((2, hd)) for hd in gr] + pad, 0).astype(BF16)
            st['s', gi_] = _dot_nt(q, k)

        def softmax(gi_):
            f = fill[0:L * len(groups[gi_]), :]
            sc = jnp.where(f < 0.0, f, st.pop(('s', gi_)) * scale)
            e = jnp.exp(sc - jnp.max(sc, axis=1, keepdims=True))
            st['p', gi_] = e / jnp.sum(e, axis=1, keepdims=True)

        def values(gi_):
            o = _dot(st.pop(('p', gi_)), st.pop(('v', gi_)))
            for j, hd in enumerate(groups[gi_]):
                oc[:, hd * LANE:(hd + 1) * LANE] = o[L * j:L * (j + 1)]
            done.update(groups[gi_])

        def out_proj(h0, h1):
            a, b = h0 * LANE, h1 * LANE
            tok = st.pop(('tok', slot), None)
            t = jnp.concatenate(
                [_dot(oc[:, a:b], _after(wo[c, a:b, :], tok if c == 0 else None))
                 for c in range(ND)], 1)
            st['acc'] = st['acc'] + t if 'acc' in st else t

        def next_ln(_):
            r1 = pl.multiple_of(jnp.minimum(s + 1, nseg - 1) * SEG, SEG)
            ln = _layernorm(x[pl.ds(r1, SEG), :])
            hbuf[M:L, :] = ln
            st['tok', 3 * H + 24] = token(
                s >> 16, *[ln[a:a + 8, D - LANE:] for a in range(0, SEG, 8)])

        def prev_finish(_):
            ln = finish_segment(jnp.maximum(s - 1, 0))
            st['tok', 11] = token(s >> 16, *[ln[a:a + 8, D - LANE:] for a in range(0, SEG, 8)])

        events, done = {}, set()
        for gi_, gr in enumerate(groups):
            last = 3 * (gr[-1] + 1) - 1
            for delay, fn in ((0, scores), (3, softmax), (9, values)):
                events.setdefault(last + delay, []).append((fn, gi_))
        events.setdefault(0, []).append((prev_finish, 0))
        events.setdefault(3 * H + 16, []).append((next_ln, 0))
        slot = 0

        def tick():
            nonlocal slot
            for fn, a in events.pop(slot, []):
                fn(a)
            slot += 1

        for gr in groups:
            for i in (1, 0, 2):
                for hd in gr:
                    proj(i, hd)
                    tick()
        WC = 4
        for h0 in range(0, H, WC):
            while not done.issuperset(range(h0, h0 + WC)):
                tick()
            out_proj(h0, h0 + WC)
            for _ in range(WC):
                tick()
        assert not events and set(st) == {'acc'}
        hbuf[0:M, :] = st['acc'][0:M]
        otok[...] = st['acc'][M:L]

    def layer_a(layer):
        hbuf[0:M, :] = mem0[...].astype(F32)
        hbuf[M:L, :] = _layernorm(x[0:SEG, :])

        @pl.loop(0, nseg // UA)
        def _(j):
            @pl.when((layer == 0) & (j == 1))
            def _():
                cp_x2.wait()
                for cp in cp_b:
                    cp.start()

                @pl.loop(1, S // CH)
                def _(i):
                    rs = pl.ds(pl.multiple_of(i * CH, CH), CH)
                    x[rs, :] = xin[rs, :].astype(F32)

            for u in range(UA):
                a_step(j * UA + u)

        finish_segment(nseg - 1)
        otok[...] = jnp.zeros(otok.shape, F32)

    RC = 16
    NCH = LANE // RC

    def chunk_rows(i, n1):
        return pl.ds(pl.multiple_of(n1 * LANE + i * RC, RC), RC)

    lane = jax.lax.broadcasted_iota(jnp.int32, (8, LANE), 1)
    HALF = LANE // 2
    IM0, MIX = NF - 1, 2 * NF - 2

    def dft_fwd(i, buf):
        xh = jnp.concatenate([xb[chunk_rows(i, n1), :] for n1 in range(R)], 0)
        for c in [c_ + o for c_ in range(NF - 1) for o in (0, IM0)] + [MIX]:
            buf[c] = _dot(xh, _after(fd[c], (yield)))

    def radix_fwd(i, buf, zero):
        for c in range(NF):
            for h in range(0, RC, 8):
                def load(n1):
                    rs = slice(n1 * RC + h, n1 * RC + h + 8)
                    if c < NF - 1:
                        im = buf[IM0 + c, rs, :]
                        return buf[c, rs, :], jnp.where(lane == 0, 0.0, im) if c == 0 else im
                    t = buf[MIX, rs, :]
                    u = pltpu.roll(jnp.where(lane == 0, buf[IM0, rs, :], t), HALF, 1)
                    return jnp.where(lane == HALF, u, t), jnp.where(lane == HALF, 0.0, u)

                r0 = pl.multiple_of(i * RC + h, 8)
                for k1, (re, im) in enumerate(_fft16([load(n1) for n1 in range(R)], -1)):
                    ya[c, k1, pl.ds(r0, 8), :] = re
                    ya[c, k1, pl.ds(LANE + r0, 8), :] = im
            yield ya[c, 0, pl.ds(pl.multiple_of(i * RC + zero, 8), 8), :]

    def filter_transpose(i):
        n_ = S // NCH
        cols = pl.ds(pl.multiple_of(i * n_, n_), n_)
        for c in range(NF):
            for src, dst in ((wrb, wrf), (wib, wif)):
                lo, hi = c * LANE, min((c + 1) * LANE, nf)
                t = src[lo:hi, cols].astype(F32)
                if hi - lo < LANE:
                    t = jnp.concatenate([t, jnp.zeros((LANE - (hi - lo), n_), F32)], 0)
                t = t.T
                dst[c, cols, :] = t
            yield t[n_ - 8:]

    def radix_inv(i, buf, zero):
        for c in range(NF):
            for h in range(0, RC, 8):
                r0 = pl.multiple_of(i * RC + h, 8)
                v = [(xa[c, k1, pl.ds(r0, 8), :], xa[c, k1, pl.ds(LANE + r0, 8), :])
                     for k1 in range(R)]
                for n1, (re, im) in enumerate(_fft16(v, +1)):
                    rs = slice(n1 * RC + h, n1 * RC + h + 8)
                    if c < NF - 1:
                        buf[c, rs, :] = re
                        buf[IM0 + c, rs, :] = im
                    else:
                        u = pltpu.roll(jnp.where(lane == HALF, re, im), HALF, 1)
                        buf[MIX, rs, :] = jnp.where(lane < HALF, re, u)
                        buf[IM0, rs, :] = jnp.where(lane == 0, u, buf[IM0, rs, :])
            yield buf[0, pl.ds(pl.multiple_of(zero, 8), 8), :]

    def out_copy(i):
        rs = pl.ds(pl.multiple_of(i * RC, RC), RC)
        return pltpu.make_async_copy(ob.at[:, rs, :], out_hbm.at[:, rs, :], sems.at[n_out + i])

    def dft_inv(i, buf, zero):
        zz = jnp.concatenate([buf[c] for c in range(ND)], 1).astype(BF16)
        for c in range(ND):
            y = _dot(zz, _after(fi[c], (yield)))
            cs = slice(c * LANE, (c + 1) * LANE)
            for n1 in range(R):
                xn = x[chunk_rows(i, n1), cs] + y[n1 * RC:(n1 + 1) * RC]
                x[chunk_rows(i, n1), cs] = xn
                ob[n1, pl.ds(pl.multiple_of(i * RC, RC), RC), cs] = xn.astype(BF16)

    def overlap(zero, mxu, *vpu):
        LAG = 2
        next(mxu)
        toks = [None] * LAG
        while True:
            vals = [v for v in (next(gen, None) for gen in vpu) if v is not None]
            toks.append(token(zero, *vals) if vals else None)
            try:
                mxu.send(toks.pop(0))
            except StopIteration:
                break

    def layer_b(layer):
        zero = layer >> 8
        overlap(zero, dft_fwd(0, bufa), filter_transpose(0))

        @pl.loop(0, NCH // 2 - 1)
        def _(j):
            overlap(zero, dft_fwd(2 * j + 1, bufb), radix_fwd(2 * j, bufa, zero),
                    filter_transpose(2 * j + 1))
            overlap(zero, dft_fwd(2 * j + 2, bufa), radix_fwd(2 * j + 1, bufb, zero),
                    filter_transpose(2 * j + 2))

        overlap(zero, dft_fwd(NCH - 1, bufb), radix_fwd(NCH - 2, bufa, zero),
                filter_transpose(NCH - 1))
        list(radix_fwd(NCH - 1, bufb, zero))
        U = 8

        @pl.loop(0, R // U)
        def _(j):
            items = [(j * U + u, c) for u in range(U) for c in range(NF)]
            z = {}
            for t in range(len(items) + 3):
                if t < len(items):
                    k1, c = items[t]
                    z[t] = _dot(g[k1], ya[c, k1].astype(BF16))
                if t >= 3:
                    k1, c = items[t - 3]
                    zt = z.pop(t - 3)
                    zr, zi = zt[0:LANE], zt[LANE:]
                    wr = wrf[c, pl.ds(k1, LANE, stride=R), :]
                    wi = wif[c, pl.ds(k1, LANE, stride=R), :]
                    zz = jnp.concatenate([zr * wr - zi * wi, zr * wi + zi * wr], 0)
                    xa[c, k1] = _dot(gi[k1], zz.astype(BF16))

        def send(i):
            @pl.when(layer == 1)
            def _():
                out_copy(i).start()

        list(radix_inv(0, bufa, zero))

        @pl.loop(0, NCH // 2 - 1)
        def _(j):
            overlap(zero, dft_inv(2 * j, bufa, zero), radix_inv(2 * j + 1, bufb, zero))
            overlap(zero, dft_inv(2 * j + 1, bufb, zero), radix_inv(2 * j + 2, bufa, zero))
            send(2 * j)
            send(2 * j + 1)

        overlap(zero, dft_inv(NCH - 2, bufa, zero), radix_inv(NCH - 1, bufb, zero))
        overlap(zero, dft_inv(NCH - 1, bufb, zero))
        send(NCH - 2)
        send(NCH - 1)

    @pl.loop(0, 2)
    def _(layer):
        layer_a(layer)

        @pl.when(layer == 0)
        def _():
            for cp in cp_b:
                cp.wait()

        layer_b(layer)

    for i in range(NCH):
        out_copy(i).wait()


@functools.partial(jax.jit, static_argnames=("A_seg_len",))
def pallas_interleave_layers__memory_aug_recurrent_mem_tr__spectral_gfnet__prompt_kernel(
    A_x, A_mem0, A_Wq, A_Wk, A_Wv, A_Wo, A_seg_len, B_x, B_w_r, B_w_i,
):
    del B_x
    B, S, D = A_x.shape
    _, H, Dh = A_Wq.shape
    M = A_mem0.shape[1]
    SEG = int(A_seg_len)
    nf = D // 2 + 1
    FP = -(-nf // LANE) * LANE
    L = M + SEG
    assert B == 1 and Dh == LANE and S == R * LANE and D % LANE == 0 and S % SEG == 0
    assert M % 8 == 0 and SEG % 16 == 0 and L <= LANE and H % 4 == 0 and D // LANE % 2 == 1
    ND, NF = D // LANE, FP // LANE
    consts = _dft_constants(S, D, FP)

    vm = pltpu.VMEM
    scratch = [
        vm((S, D), BF16),
        vm((S, D), BF16),
        vm((M, D), BF16),
        vm((3 * ND, LANE * H // 2, LANE), U32),
        vm((3 * H, D, LANE), BF16),
        vm((ND, H * Dh, LANE), BF16),
        vm((nf, S), BF16), vm((nf, S), BF16),
        vm((NF, S, LANE), F32), vm((NF, S, LANE), F32),
        vm(consts[0].shape, BF16), vm(consts[1].shape, BF16),
        vm(consts[2].shape, BF16), vm(consts[3].shape, BF16),
        vm((S, D), F32),
        vm((L, D), F32),
        vm((L, H * Dh), F32),
        vm((SEG, D), F32),
        vm((LANE // L * L, LANE), F32),
        vm((NF, R, 2 * LANE, LANE), F32),
        vm((NF, R, 2 * LANE, LANE), F32),
        vm((ND, R * 16, LANE), F32),
        vm((ND, R * 16, LANE), F32),
        vm((R, LANE, D), BF16),
        pltpu.SemaphoreType.DMA((2 + 4 * ND + 6 + LANE // 16,)),
    ]
    any_spec = pl.BlockSpec(memory_space=pltpu.HBM)
    out = pl.pallas_call(
        functools.partial(_kernel, S=S, D=D, H=H, M=M, SEG=SEG, FP=FP),
        out_shape=jax.ShapeDtypeStruct((R, LANE, D), BF16),
        in_specs=[any_spec] * 12,
        out_specs=any_spec,
        scratch_shapes=scratch,
        compiler_params=pltpu.CompilerParams(vmem_limit_bytes=110 * 2**20),
    )(A_x.reshape(S, D), A_mem0.reshape(M, D),
      A_Wq.reshape(D * H, Dh), A_Wk.reshape(D * H, Dh), A_Wv.reshape(D * H, Dh),
      A_Wo.reshape(H * Dh, D), B_w_r.T, B_w_i.T, *consts)
    return out.reshape(B, S, D)
```

```python
import functools

import jax
import jax.numpy as jnp
import numpy as np
import jax.experimental.pallas as pl
import jax.experimental.pallas.tpu as pltpu

F32, BF16, U32 = jnp.float32, jnp.bfloat16, jnp.uint32
LANE = 128
R = 16


def _dot(a, b):
    return jax.lax.dot_general(a, b, (((1,), (0,)), ((), ())), preferred_element_type=F32)


def _dot_nt(a, b):
    return jax.lax.dot_general(a, b, (((1,), (1,)), ((), ())), preferred_element_type=F32)


def _layernorm(x):
    inv = 1.0 / x.shape[-1]
    c = x - jnp.sum(x, axis=-1, keepdims=True) * inv
    v = jnp.sum(c * c, axis=-1, keepdims=True) * inv
    return c * jax.lax.rsqrt(v + 1e-5)


def _after(w, token):
    if token is None:
        return w
    head = pltpu.bitcast(pltpu.bitcast(w[0:16], U32) | token, BF16)
    return jnp.concatenate([head, w[16:]], 0)


def _dft_constants(S, D, FP):
    nf = D // 2 + 1
    d = np.arange(D)[:, None]
    k = np.arange(nf)[None, :]
    ang = 2.0 * np.pi * ((d * k) % D) / D
    cos, sin = np.cos(ang), np.sin(ang)
    n0 = FP - LANE
    ck = np.full((nf,), 2.0)
    ck[0] = ck[D // 2] = 1.0

    def pack(re, im):
        return np.concatenate(
            [re[:, :n0], re[:, D // 2:], im[:, 1:n0], re[:, n0:D // 2], im[:, n0:D // 2]], 1)

    fwd = pack(cos, -sin)
    inv = pack(cos * ck / D, -sin * ck / D).T
    k1 = np.arange(R)[:, None, None]
    k2 = np.arange(LANE)[None, :, None]
    n2 = np.arange(LANE)[None, None, :]
    a = 2.0 * np.pi * ((n2 * (k1 + R * k2)) % S) / S
    c, s = np.cos(a), np.sin(a)
    g = np.concatenate([np.concatenate([c, s], 2), np.concatenate([-s, c], 2)], 1)
    gi = np.transpose(g, (0, 2, 1)) / S
    slab = lambda m: np.ascontiguousarray(
        m.reshape(m.shape[0], -1, LANE).transpose(1, 0, 2)).astype(BF16)
    return slab(fwd), slab(inv), g.astype(BF16), gi.astype(BF16)


def _fft4(x, sign):
    (ar, ai), (br, bi), (cr, ci), (dr, di) = x
    sr, si, tr, ti = ar + cr, ai + ci, ar - cr, ai - ci
    ur, ui, vr, vi = br + dr, bi + di, br - dr, bi - di
    p, m = (tr - vi, ti + vr), (tr + vi, ti - vr)
    y1, y3 = (p, m) if sign > 0 else (m, p)
    return [(sr + ur, si + ui), y1, (sr - ur, si - ui), y3]


def _twiddle16(z, e, sign):
    r, i = z
    if e == 0:
        return z
    if e == 4:
        return (-i, r) if sign > 0 else (i, -r)
    c = float(np.cos(2 * np.pi * e / 16))
    s = float(sign * np.sin(2 * np.pi * e / 16))
    if e % 4 == 2:
        sg = s / c
        return ((r - i) * c, (i + r) * c) if sg > 0 else ((r + i) * c, (i - r) * c)
    return (r * c - i * s, i * c + r * s)


def _fft16(x, sign):
    t = [_fft4([x[b + 4 * a] for a in range(4)], sign) for b in range(4)]
    y = [None] * 16
    for k1 in range(4):
        o = _fft4([_twiddle16(t[b][k1], b * k1, sign) for b in range(4)], sign)
        for k2 in range(4):
            y[k1 + 4 * k2] = o[k2]
    return y


def _kernel(x_hbm, mem_hbm, wq_hbm, wk_hbm, wv_hbm, wo_hbm, wr_hbm, wi_hbm,
            fd_hbm, fi_hbm, g_hbm, gi_hbm, out_hbm,
            xin, xb, mem0, stage, wqkv, wo, wrb, wib, wrf, wif, fd, fi, g, gi,
            x, hbuf, oc, otok, fill, xa, ya, bufa, bufb, ob, sems, *, S, D, H, M, SEG, FP):
    L = M + SEG
    nseg = S // SEG
    ND = D // LANE
    NF = FP // LANE
    nf = D // 2 + 1
    G = LANE // L
    groups = [list(range(a, min(a + G, H))) for a in range(0, H, G)]
    scale = LANE ** -0.5
    UA = 3
    CH = 8 * SEG
    assert (nseg - 1) % UA == 0 and (UA + 2) * SEG <= CH

    rows = LANE * H // 2
    cp_x = pltpu.make_async_copy(x_hbm.at[0:CH], xb.at[0:CH], sems.at[0])
    cp_x2 = pltpu.make_async_copy(x_hbm.at[CH:S], xin.at[CH:S], sems.at[0])
    cp_mem = pltpu.make_async_copy(mem_hbm, mem0, sems.at[1])
    cp_w = [pltpu.make_async_copy(w.bitcast(U32).at[pl.ds(c * rows, rows)], stage.at[i * ND + c],
                                  sems.at[2 + i * ND + c])
            for i, w in enumerate((wq_hbm, wk_hbm, wv_hbm)) for c in range(ND)]
    n = 2 + 3 * ND
    cp_wo = [pltpu.make_async_copy(wo_hbm.at[:, pl.ds(c * LANE, LANE)], wo.at[c], sems.at[n + c])
             for c in range(ND)]
    n += ND
    cp_b = [pltpu.make_async_copy(a, b, sems.at[n + i]) for i, (a, b) in enumerate(
        ((wr_hbm, wrb), (wi_hbm, wib), (fd_hbm, fd), (fi_hbm, fi), (g_hbm, g), (gi_hbm, gi)))]
    n_out = n + len(cp_b)
    queue = cp_w + cp_wo
    DEPTH = 4
    for cp in [cp_x, cp_mem] + queue[:DEPTH]:
        cp.start()

    r = jax.lax.broadcasted_iota(jnp.int32, fill.shape, 0)
    c = jax.lax.broadcasted_iota(jnp.int32, fill.shape, 1)
    rb = sum((r >= L * j).astype(jnp.int32) for j in range(1, G + 1))
    cb = sum((c >= L * j).astype(jnp.int32) for j in range(1, G + 1))
    ri, ci = r - L * rb, c - L * cb
    fill[...] = jnp.where(rb == cb, jnp.where((ri < M) | (ri >= ci), 0.0, -1e9),
                          -jnp.inf).astype(F32)
    otok[...] = jnp.zeros(otok.shape, F32)

    cp_x.wait()
    x[0:CH, :] = xb[0:CH, :].astype(F32)
    cp_mem.wait()

    for t, cp in enumerate(cp_w):
        cp.wait()
        queue[t + DEPTH].start()
        i, c = divmod(t, ND)

        @pl.loop(0, H // 2)
        def _(j):
            w = stage[t, pl.ds(j, LANE, stride=H // 2), :]
            lo = pltpu.bitcast(w << 16, F32).astype(BF16)
            hi = pltpu.bitcast(w & np.uint32(0xFFFF0000), F32).astype(BF16)
            wqkv[i * H + 2 * j, c * LANE:(c + 1) * LANE, :] = lo
            wqkv[i * H + 2 * j + 1, c * LANE:(c + 1) * LANE, :] = hi

    for cp in queue[len(cp_w) + DEPTH:]:
        cp.start()

    def token(zero, *vals):
        bits = functools.reduce(jnp.bitwise_or, [pltpu.bitcast(v, U32) for v in vals])
        return bits & zero.astype(U32)

    def finish_segment(s):
        r0 = pl.multiple_of(s * SEG, SEG)
        xn = x[pl.ds(r0, SEG), :] + otok[...]
        x[pl.ds(r0, SEG), :] = xn
        ln = _layernorm(xn)
        xb[pl.ds(r0, SEG), :] = ln.astype(BF16)
        return ln

    def a_step(s, before_out_proj=None):
        st = {}

        def proj(i, hd):
            st[i, hd] = _dot(hbuf[...], _after(wqkv[i * H + hd], st.pop(('tok', slot), None)))

        def scores(gi_):
            gr = groups[gi_]
            pad = [jnp.zeros((LANE - L * len(gr), LANE), F32)]
            q = jnp.concatenate([st.pop((0, hd)) for hd in gr], 0)
            k = jnp.concatenate([st.pop((1, hd)) for hd in gr] + pad, 0).astype(BF16)
            st['v', gi_] = jnp.concatenate([st.pop((2, hd)) for hd in gr] + pad, 0).astype(BF16)
            st['s', gi_] = _dot_nt(q, k)

        def softmax(gi_):
            f = fill[0:L * len(groups[gi_]), :]
            sc = jnp.where(f < 0.0, f, st.pop(('s', gi_)) * scale)
            e = jnp.exp(sc - jnp.max(sc, axis=1, keepdims=True))
            st['p', gi_] = e / jnp.sum(e, axis=1, keepdims=True)

        def values(gi_):
            o = _dot(st.pop(('p', gi_)), st.pop(('v', gi_)))
            for j, hd in enumerate(groups[gi_]):
                oc[:, hd * LANE:(hd + 1) * LANE] = o[L * j:L * (j + 1)]
            done.update(groups[gi_])

        def out_proj(h0, h1):
            a, b = h0 * LANE, h1 * LANE
            tok = st.pop(('tok', slot), None)
            t = jnp.concatenate(
                [_dot(oc[:, a:b], _after(wo[c, a:b, :], tok if c == 0 else None))
                 for c in range(ND)], 1)
            st['acc'] = st['acc'] + t if 'acc' in st else t

        def next_ln(_):
            r1 = pl.multiple_of(jnp.minimum(s + 1, nseg - 1) * SEG, SEG)
            ln = _layernorm(x[pl.ds(r1, SEG), :])
            hbuf[M:L, :] = ln
            st['tok', 3 * H + 24] = token(
                s >> 16, *[ln[a:a + 8, D - LANE:] for a in range(0, SEG, 8)])

        def prev_finish(_):
            ln = finish_segment(jnp.maximum(s - 1, 0))
            st['tok', 11] = token(s >> 16, *[ln[a:a + 8, D - LANE:] for a in range(0, SEG, 8)])

        events, done = {}, set()
        for gi_, gr in enumerate(groups):
            last = 3 * (gr[-1] + 1) - 1
            for delay, fn in ((0, scores), (3, softmax), (9, values)):
                events.setdefault(last + delay, []).append((fn, gi_))
        events.setdefault(0, []).append((prev_finish, 0))
        events.setdefault(3 * H + 16, []).append((next_ln, 0))
        slot = 0

        def tick():
            nonlocal slot
            for fn, a in events.pop(slot, []):
                fn(a)
            slot += 1

        for gr in groups:
            for i in (1, 0, 2):
                for hd in gr:
                    proj(i, hd)
                    tick()
        WC = 4
        if before_out_proj is not None:
            before_out_proj()
        for h0 in range(0, H, WC):
            while not done.issuperset(range(h0, h0 + WC)):
                tick()
            out_proj(h0, h0 + WC)
            for _ in range(WC):
                tick()
        assert not events and set(st) == {'acc'}
        hbuf[0:M, :] = st['acc'][0:M]
        otok[...] = st['acc'][M:L]

    def layer_a(layer):
        hbuf[0:M, :] = mem0[...].astype(F32)
        hbuf[M:L, :] = _layernorm(x[0:SEG, :])

        def wait_wo():
            @pl.when(layer == 0)
            def _():
                for cp in cp_wo:
                    cp.wait()
                cp_x2.start()

        a_step(layer >> 8, wait_wo)

        @pl.loop(0, (nseg - 1) // UA)
        def _(j):
            @pl.when((layer == 0) & (j == 1))
            def _():
                cp_x2.wait()
                for cp in cp_b:
                    cp.start()

                @pl.loop(1, S // CH)
                def _(i):
                    rs = pl.ds(pl.multiple_of(i * CH, CH), CH)
                    x[rs, :] = xin[rs, :].astype(F32)

            for u in range(UA):
                a_step(1 + j * UA + u)

        finish_segment(nseg - 1)
        otok[...] = jnp.zeros(otok.shape, F32)

    RC = 16
    NCH = LANE // RC

    def chunk_rows(i, n1):
        return pl.ds(n1 * LANE + i * RC, RC)

    lane = jax.lax.broadcasted_iota(jnp.int32, (8, LANE), 1)
    HALF = LANE // 2
    IM0, MIX = NF - 1, 2 * NF - 2

    def dft_fwd(i, buf):
        xh = jnp.concatenate([xb[chunk_rows(i, n1), :] for n1 in range(R)], 0)
        for c in [c_ + o for c_ in range(NF - 1) for o in (0, IM0)] + [MIX]:
            buf[c] = _dot(xh, _after(fd[c], (yield)))

    def radix_fwd(i, buf, zero):
        for c in range(NF):
            for h in range(0, RC, 8):
                def load(n1):
                    rs = slice(n1 * RC + h, n1 * RC + h + 8)
                    if c < NF - 1:
                        im = buf[IM0 + c, rs, :]
                        return buf[c, rs, :], jnp.where(lane == 0, 0.0, im) if c == 0 else im
                    t = buf[MIX, rs, :]
                    u = pltpu.roll(jnp.where(lane == 0, buf[IM0, rs, :], t), HALF, 1)
                    return jnp.where(lane == HALF, u, t), jnp.where(lane == HALF, 0.0, u)

                r0 = i * RC + h
                for k1, (re, im) in enumerate(_fft16([load(n1) for n1 in range(R)], -1)):
                    ya[c, k1, pl.ds(r0, 8), :] = re
                    ya[c, k1, pl.ds(LANE + r0, 8), :] = im
            yield ya[c, 0, pl.ds(pl.multiple_of(i * RC + zero, 8), 8), :]

    def filter_transpose(i):
        n_ = S // NCH
        cols = pl.ds(i * n_, n_)
        for c in range(NF):
            for src, dst in ((wrb, wrf), (wib, wif)):
                lo, hi = c * LANE, min((c + 1) * LANE, nf)
                t = src[lo:hi, cols].astype(F32)
                if hi - lo < LANE:
                    t = jnp.concatenate([t, jnp.zeros((LANE - (hi - lo), n_), F32)], 0)
                t = t.T
                dst[c, cols, :] = t
            yield t[n_ - 8:]

    def radix_inv(i, buf, zero):
        for c in range(NF):
            for h in range(0, RC, 8):
                r0 = i * RC + h
                v = [(xa[c, k1, pl.ds(r0, 8), :], xa[c, k1, pl.ds(LANE + r0, 8), :])
                     for k1 in range(R)]
                for n1, (re, im) in enumerate(_fft16(v, +1)):
                    rs = slice(n1 * RC + h, n1 * RC + h + 8)
                    if c < NF - 1:
                        buf[c, rs, :] = re
                        buf[IM0 + c, rs, :] = im
                    else:
                        u = pltpu.roll(jnp.where(lane == HALF, re, im), HALF, 1)
                        buf[MIX, rs, :] = jnp.where(lane < HALF, re, u)
                        buf[IM0, rs, :] = jnp.where(lane == 0, u, buf[IM0, rs, :])
            yield buf[0, pl.ds(pl.multiple_of(zero, 8), 8), :]

    def out_copy(i):
        rs = pl.ds(i * RC, RC)
        return pltpu.make_async_copy(ob.at[:, rs, :], out_hbm.at[:, rs, :], sems.at[n_out + i])

    def dft_inv(i, buf):
        zz = jnp.concatenate([buf[c] for c in range(ND)], 1).astype(BF16)
        for c in range(ND):
            y = _dot(zz, _after(fi[c], (yield)))
            cs = slice(c * LANE, (c + 1) * LANE)
            for n1 in range(R):
                xn = x[chunk_rows(i, n1), cs] + y[n1 * RC:(n1 + 1) * RC]
                x[chunk_rows(i, n1), cs] = xn
                ob[n1, pl.ds(i * RC, RC), cs] = xn.astype(BF16)

    def overlap(zero, mxu, *vpu):
        LAG = 2
        next(mxu)
        toks = [None] * LAG
        while True:
            vals = [v for v in (next(gen, None) for gen in vpu) if v is not None]
            toks.append(token(zero, *vals) if vals else None)
            try:
                mxu.send(toks.pop(0))
            except StopIteration:
                break

    def layer_b(layer):
        zero = layer >> 8
        bufs = (bufa, bufb)
        overlap(zero, dft_fwd(0, bufa), filter_transpose(0))
        for i in range(1, NCH):
            overlap(zero, dft_fwd(i, bufs[i % 2]), radix_fwd(i - 1, bufs[1 - i % 2], zero),
                    filter_transpose(i))
        list(radix_fwd(NCH - 1, bufb, zero))
        U = 8

        @pl.loop(0, R // U)
        def _(j):
            items = [(j * U + u, c) for u in range(U) for c in range(NF)]
            z = {}
            for t in range(len(items) + 3):
                if t < len(items):
                    k1, c = items[t]
                    z[t] = _dot(g[k1], ya[c, k1].astype(BF16))
                if t >= 3:
                    k1, c = items[t - 3]
                    zt = z.pop(t - 3)
                    zr, zi = zt[0:LANE], zt[LANE:]
                    wr = wrf[c, pl.ds(k1, LANE, stride=R), :]
                    wi = wif[c, pl.ds(k1, LANE, stride=R), :]
                    zz = jnp.concatenate([zr * wr - zi * wi, zr * wi + zi * wr], 0)
                    xa[c, k1] = _dot(gi[k1], zz.astype(BF16))

        @pl.when(layer == 1)
        def _():
            for i in range(NCH):
                out_copy(i).wait()

        list(radix_inv(0, bufa, zero))
        for i in range(NCH):
            nxt = [radix_inv(i + 1, bufs[1 - i % 2], zero)] if i + 1 < NCH else []
            overlap(zero, dft_inv(i, bufs[i % 2]), *nxt)
            out_copy(i).start()

    @pl.loop(0, 2)
    def _(layer):
        layer_a(layer)

        @pl.when(layer == 0)
        def _():
            for cp in cp_b:
                cp.wait()

        layer_b(layer)

    for i in range(NCH):
        out_copy(i).wait()


@functools.partial(jax.jit, static_argnames=("A_seg_len",))
def pallas_interleave_layers__memory_aug_recurrent_mem_tr__spectral_gfnet__prompt_kernel(
    A_x, A_mem0, A_Wq, A_Wk, A_Wv, A_Wo, A_seg_len, B_x, B_w_r, B_w_i,
):
    del B_x
    B, S, D = A_x.shape
    _, H, Dh = A_Wq.shape
    M = A_mem0.shape[1]
    SEG = int(A_seg_len)
    nf = D // 2 + 1
    FP = -(-nf // LANE) * LANE
    L = M + SEG
    assert B == 1 and Dh == LANE and S == R * LANE and D % LANE == 0 and S % SEG == 0
    assert M % 8 == 0 and SEG % 16 == 0 and L <= LANE and H % 4 == 0 and D // LANE % 2 == 1
    ND, NF = D // LANE, FP // LANE
    consts = _dft_constants(S, D, FP)

    vm = pltpu.VMEM
    scratch = [
        vm((S, D), BF16),
        vm((S, D), BF16),
        vm((M, D), BF16),
        vm((3 * ND, LANE * H // 2, LANE), U32),
        vm((3 * H, D, LANE), BF16),
        vm((ND, H * Dh, LANE), BF16),
        vm((nf, S), BF16), vm((nf, S), BF16),
        vm((NF, S, LANE), F32), vm((NF, S, LANE), F32),
        vm(consts[0].shape, BF16), vm(consts[1].shape, BF16),
        vm(consts[2].shape, BF16), vm(consts[3].shape, BF16),
        vm((S, D), F32),
        vm((L, D), F32),
        vm((L, H * Dh), F32),
        vm((SEG, D), F32),
        vm((LANE // L * L, LANE), F32),
        vm((NF, R, 2 * LANE, LANE), F32),
        vm((NF, R, 2 * LANE, LANE), F32),
        vm((ND, R * 16, LANE), F32),
        vm((ND, R * 16, LANE), F32),
        vm((R, LANE, D), BF16),
        pltpu.SemaphoreType.DMA((2 + 4 * ND + 6 + LANE // 16,)),
    ]
    any_spec = pl.BlockSpec(memory_space=pltpu.HBM)
    out = pl.pallas_call(
        functools.partial(_kernel, S=S, D=D, H=H, M=M, SEG=SEG, FP=FP),
        out_shape=jax.ShapeDtypeStruct((R, LANE, D), BF16),
        in_specs=[any_spec] * 12,
        out_specs=any_spec,
        scratch_shapes=scratch,
        compiler_params=pltpu.CompilerParams(vmem_limit_bytes=110 * 2**20),
    )(A_x.reshape(S, D), A_mem0.reshape(M, D),
      A_Wq.reshape(D * H, Dh), A_Wk.reshape(D * H, Dh), A_Wv.reshape(D * H, Dh),
      A_Wo.reshape(H * Dh, D), B_w_r.T, B_w_i.T, *consts)
    return out.reshape(B, S, D)
```

```python
import functools

import jax
import jax.numpy as jnp
import numpy as np
import jax.experimental.pallas as pl
import jax.experimental.pallas.tpu as pltpu

F32, BF16, U32 = jnp.float32, jnp.bfloat16, jnp.uint32
LANE = 128
R = 16


def _dot(a, b):
    return jax.lax.dot_general(a, b, (((1,), (0,)), ((), ())), preferred_element_type=F32)


def _dot_nt(a, b):
    return jax.lax.dot_general(a, b, (((1,), (1,)), ((), ())), preferred_element_type=F32)


def _layernorm(x):
    inv = 1.0 / x.shape[-1]
    c = x - jnp.sum(x, axis=-1, keepdims=True) * inv
    v = jnp.sum(c * c, axis=-1, keepdims=True) * inv
    return c * jax.lax.rsqrt(v + 1e-5)


def _after(w, token):
    if token is None:
        return w
    head = pltpu.bitcast(pltpu.bitcast(w[0:16], U32) | token, BF16)
    return jnp.concatenate([head, w[16:]], 0)


def _dft_constants(S, D, FP):
    nf = D // 2 + 1
    d = np.arange(D)[:, None]
    k = np.arange(nf)[None, :]
    ang = 2.0 * np.pi * ((d * k) % D) / D
    cos, sin = np.cos(ang), np.sin(ang)
    n0 = FP - LANE
    ck = np.full((nf,), 2.0)
    ck[0] = ck[D // 2] = 1.0

    def pack(re, im):
        return np.concatenate(
            [re[:, :n0], re[:, D // 2:], im[:, 1:n0], re[:, n0:D // 2], im[:, n0:D // 2]], 1)

    fwd = pack(cos, -sin)
    inv = pack(cos * ck / D, -sin * ck / D).T
    k1 = np.arange(R)[:, None, None]
    k2 = np.arange(LANE)[None, :, None]
    n2 = np.arange(LANE)[None, None, :]
    a = 2.0 * np.pi * ((n2 * (k1 + R * k2)) % S) / S
    c, s = np.cos(a), np.sin(a)
    g = np.concatenate([np.concatenate([c, s], 2), np.concatenate([-s, c], 2)], 1)
    gi = np.transpose(g, (0, 2, 1)) / S
    slab = lambda m: np.ascontiguousarray(
        m.reshape(m.shape[0], -1, LANE).transpose(1, 0, 2)).astype(BF16)
    return slab(fwd), slab(inv), g.astype(BF16), gi.astype(BF16)


def _fft4(x, sign):
    (ar, ai), (br, bi), (cr, ci), (dr, di) = x
    sr, si, tr, ti = ar + cr, ai + ci, ar - cr, ai - ci
    ur, ui, vr, vi = br + dr, bi + di, br - dr, bi - di
    p, m = (tr - vi, ti + vr), (tr + vi, ti - vr)
    y1, y3 = (p, m) if sign > 0 else (m, p)
    return [(sr + ur, si + ui), y1, (sr - ur, si - ui), y3]


def _twiddle16(z, e, sign):
    r, i = z
    if e == 0:
        return z
    if e == 4:
        return (-i, r) if sign > 0 else (i, -r)
    c = float(np.cos(2 * np.pi * e / 16))
    s = float(sign * np.sin(2 * np.pi * e / 16))
    if e % 4 == 2:
        sg = s / c
        return ((r - i) * c, (i + r) * c) if sg > 0 else ((r + i) * c, (i - r) * c)
    return (r * c - i * s, i * c + r * s)


def _fft16(x, sign):
    t = [_fft4([x[b + 4 * a] for a in range(4)], sign) for b in range(4)]
    y = [None] * 16
    for k1 in range(4):
        o = _fft4([_twiddle16(t[b][k1], b * k1, sign) for b in range(4)], sign)
        for k2 in range(4):
            y[k1 + 4 * k2] = o[k2]
    return y


def _kernel(x_hbm, mem_hbm, wq_hbm, wk_hbm, wv_hbm, wo_hbm, wr_hbm, wi_hbm,
            fd_hbm, fi_hbm, g_hbm, gi_hbm, out_hbm,
            xin, xb, mem0, stage, wqkv, wo, wrb, wib, wrf, wif, fd, fi, g, gi,
            x, hbuf, oc, otok, fill, xa, ya, bufa, bufb, bufc, bufd, ob, sems, *, S, D, H, M, SEG, FP):
    L = M + SEG
    nseg = S // SEG
    ND = D // LANE
    NF = FP // LANE
    nf = D // 2 + 1
    G = LANE // L
    groups = [list(range(a, min(a + G, H))) for a in range(0, H, G)]
    scale = LANE ** -0.5
    UA = 3
    CH = 8 * SEG
    assert (nseg - 1) % UA == 0 and (UA + 2) * SEG <= CH

    rows = LANE * H // 2
    cp_x = pltpu.make_async_copy(x_hbm.at[0:CH], xb.at[0:CH], sems.at[0])
    cp_x2 = pltpu.make_async_copy(x_hbm.at[CH:S], xin.at[CH:S], sems.at[0])
    cp_mem = pltpu.make_async_copy(mem_hbm, mem0, sems.at[1])
    cp_w = [pltpu.make_async_copy(w.bitcast(U32).at[pl.ds(c * rows, rows)], stage.at[i * ND + c],
                                  sems.at[2 + i * ND + c])
            for i, w in enumerate((wq_hbm, wk_hbm, wv_hbm)) for c in range(ND)]
    n = 2 + 3 * ND
    cp_wo = [pltpu.make_async_copy(wo_hbm.at[:, pl.ds(c * LANE, LANE)], wo.at[c], sems.at[n + c])
             for c in range(ND)]
    n += ND
    cp_b = [pltpu.make_async_copy(a, b, sems.at[n + i]) for i, (a, b) in enumerate(
        ((wr_hbm, wrb), (wi_hbm, wib), (fd_hbm, fd), (fi_hbm, fi), (g_hbm, g), (gi_hbm, gi)))]
    n_out = n + len(cp_b)
    queue = cp_w + cp_wo
    DEPTH = 4
    for cp in [cp_x, cp_mem] + queue[:DEPTH]:
        cp.start()

    r = jax.lax.broadcasted_iota(jnp.int32, fill.shape, 0)
    c = jax.lax.broadcasted_iota(jnp.int32, fill.shape, 1)
    rb = sum((r >= L * j).astype(jnp.int32) for j in range(1, G + 1))
    cb = sum((c >= L * j).astype(jnp.int32) for j in range(1, G + 1))
    ri, ci = r - L * rb, c - L * cb
    fill[...] = jnp.where(rb == cb, jnp.where((ri < M) | (ri >= ci), 0.0, -1e9),
                          -jnp.inf).astype(F32)
    otok[...] = jnp.zeros(otok.shape, F32)

    cp_x.wait()
    x[0:CH, :] = xb[0:CH, :].astype(F32)
    cp_mem.wait()

    for t, cp in enumerate(cp_w):
        cp.wait()
        queue[t + DEPTH].start()
        i, c = divmod(t, ND)

        @pl.loop(0, H // 2)
        def _(j):
            w = stage[t, pl.ds(j, LANE, stride=H // 2), :]
            lo = pltpu.bitcast(w << 16, F32).astype(BF16)
            hi = pltpu.bitcast(w & np.uint32(0xFFFF0000), F32).astype(BF16)
            wqkv[i * H + 2 * j, c * LANE:(c + 1) * LANE, :] = lo
            wqkv[i * H + 2 * j + 1, c * LANE:(c + 1) * LANE, :] = hi

    for cp in queue[len(cp_w) + DEPTH:]:
        cp.start()

    def token(zero, *vals):
        bits = functools.reduce(jnp.bitwise_or, [pltpu.bitcast(v, U32) for v in vals])
        return bits & zero.astype(U32)

    def finish_segment(s):
        r0 = pl.multiple_of(s * SEG, SEG)
        xn = x[pl.ds(r0, SEG), :] + otok[...]
        x[pl.ds(r0, SEG), :] = xn
        ln = _layernorm(xn)
        xb[pl.ds(r0, SEG), :] = ln.astype(BF16)
        return ln

    def a_step(s, before_out_proj=None):
        st = {}

        def proj(i, hd):
            st[i, hd] = _dot(hbuf[...], _after(wqkv[i * H + hd], st.pop(('tok', slot), None)))

        def scores(gi_):
            gr = groups[gi_]
            pad = [jnp.zeros((LANE - L * len(gr), LANE), F32)]
            q = jnp.concatenate([st.pop((0, hd)) for hd in gr], 0)
            k = jnp.concatenate([st.pop((1, hd)) for hd in gr] + pad, 0).astype(BF16)
            st['v', gi_] = jnp.concatenate([st.pop((2, hd)) for hd in gr] + pad, 0).astype(BF16)
            st['s', gi_] = _dot_nt(q, k)

        def softmax(gi_):
            f = fill[0:L * len(groups[gi_]), :]
            sc = jnp.where(f < 0.0, f, st.pop(('s', gi_)) * scale)
            e = jnp.exp(sc - jnp.max(sc, axis=1, keepdims=True))
            st['p', gi_] = e / jnp.sum(e, axis=1, keepdims=True)

        def values(gi_):
            o = _dot(st.pop(('p', gi_)), st.pop(('v', gi_)))
            for j, hd in enumerate(groups[gi_]):
                oc[:, hd * LANE:(hd + 1) * LANE] = o[L * j:L * (j + 1)]
            done.update(groups[gi_])

        def out_proj(h0, h1):
            a, b = h0 * LANE, h1 * LANE
            tok = st.pop(('tok', slot), None)
            t = jnp.concatenate(
                [_dot(oc[:, a:b], _after(wo[c, a:b, :], tok if c == 0 else None))
                 for c in range(ND)], 1)
            st['acc'] = st['acc'] + t if 'acc' in st else t

        def next_ln(_):
            r1 = pl.multiple_of(jnp.minimum(s + 1, nseg - 1) * SEG, SEG)
            ln = _layernorm(x[pl.ds(r1, SEG), :])
            hbuf[M:L, :] = ln
            st['tok', 3 * H + 24] = token(
                s >> 16, *[ln[a:a + 8, D - LANE:] for a in range(0, SEG, 8)])

        def prev_finish(_):
            ln = finish_segment(jnp.maximum(s - 1, 0))
            st['tok', 11] = token(s >> 16, *[ln[a:a + 8, D - LANE:] for a in range(0, SEG, 8)])

        events, done = {}, set()
        for gi_, gr in enumerate(groups):
            last = 3 * (gr[-1] + 1) - 1
            for delay, fn in ((0, scores), (3, softmax), (9, values)):
                events.setdefault(last + delay, []).append((fn, gi_))
        events.setdefault(0, []).append((prev_finish, 0))
        events.setdefault(3 * H + 16, []).append((next_ln, 0))
        slot = 0

        def tick():
            nonlocal slot
            for fn, a in events.pop(slot, []):
                fn(a)
            slot += 1

        for gr in groups:
            for i in (1, 0, 2):
                for hd in gr:
                    proj(i, hd)
                    tick()
        WC = 4
        if before_out_proj is not None:
            before_out_proj()
        for h0 in range(0, H, WC):
            while not done.issuperset(range(h0, h0 + WC)):
                tick()
            out_proj(h0, h0 + WC)
            for _ in range(WC):
                tick()
        assert not events and set(st) == {'acc'}
        hbuf[0:M, :] = st['acc'][0:M]
        otok[...] = st['acc'][M:L]

    def layer_a(layer):
        hbuf[0:M, :] = mem0[...].astype(F32)
        hbuf[M:L, :] = _layernorm(x[0:SEG, :])

        def wait_wo():
            @pl.when(layer == 0)
            def _():
                for cp in cp_wo:
                    cp.wait()
                cp_x2.start()

        a_step(layer >> 8, wait_wo)

        @pl.loop(0, (nseg - 1) // UA)
        def _(j):
            @pl.when((layer == 0) & (j == 1))
            def _():
                cp_x2.wait()
                for cp in cp_b:
                    cp.start()

                @pl.loop(1, S // CH)
                def _(i):
                    rs = pl.ds(pl.multiple_of(i * CH, CH), CH)
                    x[rs, :] = xin[rs, :].astype(F32)

            for u in range(UA):
                a_step(1 + j * UA + u)

        finish_segment(nseg - 1)
        otok[...] = jnp.zeros(otok.shape, F32)

    RC = 16
    NCH = LANE // RC

    def chunk_rows(i, n1):
        return pl.ds(n1 * LANE + i * RC, RC)

    lane = jax.lax.broadcasted_iota(jnp.int32, (8, LANE), 1)
    HALF = LANE // 2
    IM0, MIX = NF - 1, 2 * NF - 2

    def dft_fwd(i, buf):
        xh = jnp.concatenate([xb[chunk_rows(i, n1), :] for n1 in range(R)], 0)
        for c in [c_ + o for c_ in range(NF - 1) for o in (0, IM0)] + [MIX]:
            buf[c] = _dot(xh, _after(fd[c], (yield)))

    def radix_fwd(i, buf, zero):
        for c in range(NF):
            for h in range(0, RC, 8):
                def load(n1):
                    rs = slice(n1 * RC + h, n1 * RC + h + 8)
                    if c < NF - 1:
                        im = buf[IM0 + c, rs, :]
                        return buf[c, rs, :], jnp.where(lane == 0, 0.0, im) if c == 0 else im
                    t = buf[MIX, rs, :]
                    u = pltpu.roll(jnp.where(lane == 0, buf[IM0, rs, :], t), HALF, 1)
                    return jnp.where(lane == HALF, u, t), jnp.where(lane == HALF, 0.0, u)

                r0 = i * RC + h
                for k1, (re, im) in enumerate(_fft16([load(n1) for n1 in range(R)], -1)):
                    ya[c, k1, pl.ds(r0, 8), :] = re
                    ya[c, k1, pl.ds(LANE + r0, 8), :] = im
            yield ya[c, 0, pl.ds(pl.multiple_of(i * RC + zero, 8), 8), :]

    def filter_transpose(i):
        n_ = S // NCH
        cols = pl.ds(i * n_, n_)
        for c in range(NF):
            for src, dst in ((wrb, wrf), (wib, wif)):
                lo, hi = c * LANE, min((c + 1) * LANE, nf)
                t = src[lo:hi, cols].astype(F32)
                if hi - lo < LANE:
                    t = jnp.concatenate([t, jnp.zeros((LANE - (hi - lo), n_), F32)], 0)
                t = t.T
                dst[c, cols, :] = t
            yield t[n_ - 8:]

    def radix_inv(i, buf, zero):
        for c in range(NF):
            for h in range(0, RC, 8):
                r0 = i * RC + h
                v = [(xa[c, k1, pl.ds(r0, 8), :], xa[c, k1, pl.ds(LANE + r0, 8), :])
                     for k1 in range(R)]
                o = _fft16(v, +1)
                rs = slice(h * R, (h + 8) * R)
                re = jnp.concatenate([z[0] for z in o], 0)
                im = jnp.concatenate([z[1] for z in o], 0)
                if c < NF - 1:
                    buf[c, rs, :] = re.astype(BF16)
                    buf[IM0 + c, rs, :] = im.astype(BF16)
                else:
                    ln = jax.lax.broadcasted_iota(jnp.int32, re.shape, 1)
                    u = pltpu.roll(jnp.where(ln == HALF, re, im), HALF, 1)
                    buf[MIX, rs, :] = jnp.where(ln < HALF, re, u).astype(BF16)
                    buf[IM0, rs, :] = jnp.where(
                        ln == 0, u, buf[IM0, rs, :].astype(F32)).astype(BF16)
            yield buf[0, pl.ds(pl.multiple_of(zero, 16), 16), :]

    def out_copy(i):
        rs = pl.ds(i * RC, RC)
        return pltpu.make_async_copy(ob.at[:, rs, :], out_hbm.at[:, rs, :], sems.at[n_out + i])

    def dft_inv(i, buf):
        zz = jnp.concatenate([buf[c] for c in range(ND)], 1)
        for c in range(ND):
            y = _dot(zz, _after(fi[c], (yield)))
            cs = slice(c * LANE, (c + 1) * LANE)
            for n1 in range(R):
                xn = x[chunk_rows(i, n1), cs] + jnp.concatenate(
                    [y[h * R + n1 * 8:h * R + n1 * 8 + 8] for h in range(0, RC, 8)], 0)
                x[chunk_rows(i, n1), cs] = xn
                ob[n1, pl.ds(i * RC, RC), cs] = xn.astype(BF16)

    def overlap(zero, mxu, *vpu):
        LAG = 2
        next(mxu)
        toks = [None] * LAG
        while True:
            vals = [v for v in (next(gen, None) for gen in vpu) if v is not None]
            toks.append(token(zero, *vals) if vals else None)
            try:
                mxu.send(toks.pop(0))
            except StopIteration:
                break

    def layer_b(layer):
        zero = layer >> 8
        bufs = (bufa, bufb)
        overlap(zero, dft_fwd(0, bufa), filter_transpose(0))
        for i in range(1, NCH):
            overlap(zero, dft_fwd(i, bufs[i % 2]), radix_fwd(i - 1, bufs[1 - i % 2], zero),
                    filter_transpose(i))
        list(radix_fwd(NCH - 1, bufb, zero))
        U = 8

        @pl.loop(0, R // U)
        def _(j):
            items = [(j * U + u, c) for u in range(U) for c in range(NF)]
            z = {}
            for t in range(len(items) + 3):
                if t < len(items):
                    k1, c = items[t]
                    z[t] = _dot(g[k1], ya[c, k1].astype(BF16))
                if t >= 3:
                    k1, c = items[t - 3]
                    zt = z.pop(t - 3)
                    zr, zi = zt[0:LANE], zt[LANE:]
                    wr = wrf[c, pl.ds(k1, LANE, stride=R), :]
                    wi = wif[c, pl.ds(k1, LANE, stride=R), :]
                    zz = jnp.concatenate([zr * wr - zi * wi, zr * wi + zi * wr], 0)
                    xa[c, k1] = _dot(gi[k1], zz.astype(BF16))

        @pl.when(layer == 1)
        def _():
            for i in range(NCH):
                out_copy(i).wait()

        bufs = (bufc, bufd)
        list(radix_inv(0, bufc, zero))
        for i in range(NCH):
            nxt = [radix_inv(i + 1, bufs[1 - i % 2], zero)] if i + 1 < NCH else []
            overlap(zero, dft_inv(i, bufs[i % 2]), *nxt)
            out_copy(i).start()

    @pl.loop(0, 2)
    def _(layer):
        layer_a(layer)

        @pl.when(layer == 0)
        def _():
            for cp in cp_b:
                cp.wait()

        layer_b(layer)

    for i in range(NCH):
        out_copy(i).wait()


@functools.partial(jax.jit, static_argnames=("A_seg_len",))
def pallas_interleave_layers__memory_aug_recurrent_mem_tr__spectral_gfnet__prompt_kernel(
    A_x, A_mem0, A_Wq, A_Wk, A_Wv, A_Wo, A_seg_len, B_x, B_w_r, B_w_i,
):
    del B_x
    B, S, D = A_x.shape
    _, H, Dh = A_Wq.shape
    M = A_mem0.shape[1]
    SEG = int(A_seg_len)
    nf = D // 2 + 1
    FP = -(-nf // LANE) * LANE
    L = M + SEG
    assert B == 1 and Dh == LANE and S == R * LANE and D % LANE == 0 and S % SEG == 0
    assert M % 8 == 0 and SEG % 16 == 0 and L <= LANE and H % 4 == 0 and D // LANE % 2 == 1
    ND, NF = D // LANE, FP // LANE
    consts = _dft_constants(S, D, FP)

    vm = pltpu.VMEM
    scratch = [
        vm((S, D), BF16),
        vm((S, D), BF16),
        vm((M, D), BF16),
        vm((3 * ND, LANE * H // 2, LANE), U32),
        vm((3 * H, D, LANE), BF16),
        vm((ND, H * Dh, LANE), BF16),
        vm((nf, S), BF16), vm((nf, S), BF16),
        vm((NF, S, LANE), F32), vm((NF, S, LANE), F32),
        vm(consts[0].shape, BF16), vm(consts[1].shape, BF16),
        vm(consts[2].shape, BF16), vm(consts[3].shape, BF16),
        vm((S, D), F32),
        vm((L, D), F32),
        vm((L, H * Dh), F32),
        vm((SEG, D), F32),
        vm((LANE // L * L, LANE), F32),
        vm((NF, R, 2 * LANE, LANE), F32),
        vm((NF, R, 2 * LANE, LANE), F32),
        vm((ND, R * 16, LANE), F32),
        vm((ND, R * 16, LANE), F32),
        vm((ND, R * 16, LANE), BF16),
        vm((ND, R * 16, LANE), BF16),
        vm((R, LANE, D), BF16),
        pltpu.SemaphoreType.DMA((2 + 4 * ND + 6 + LANE // 16,)),
    ]
    any_spec = pl.BlockSpec(memory_space=pltpu.HBM)
    out = pl.pallas_call(
        functools.partial(_kernel, S=S, D=D, H=H, M=M, SEG=SEG, FP=FP),
        out_shape=jax.ShapeDtypeStruct((R, LANE, D), BF16),
        in_specs=[any_spec] * 12,
        out_specs=any_spec,
        scratch_shapes=scratch,
        compiler_params=pltpu.CompilerParams(vmem_limit_bytes=110 * 2**20),
    )(A_x.reshape(S, D), A_mem0.reshape(M, D),
      A_Wq.reshape(D * H, Dh), A_Wk.reshape(D * H, Dh), A_Wv.reshape(D * H, Dh),
      A_Wo.reshape(H * Dh, D), B_w_r.T, B_w_i.T, *consts)
    return out.reshape(B, S, D)
```

```python
import functools

import jax
import jax.numpy as jnp
import numpy as np
import jax.experimental.pallas as pl
import jax.experimental.pallas.tpu as pltpu

F32, BF16, U32 = jnp.float32, jnp.bfloat16, jnp.uint32
LANE = 128
R = 16


def _dot(a, b):
    return jax.lax.dot_general(a, b, (((1,), (0,)), ((), ())), preferred_element_type=F32)


def _dot_nt(a, b):
    return jax.lax.dot_general(a, b, (((1,), (1,)), ((), ())), preferred_element_type=F32)


def _layernorm(x):
    inv = 1.0 / x.shape[-1]
    c = x - jnp.sum(x, axis=-1, keepdims=True) * inv
    v = jnp.sum(c * c, axis=-1, keepdims=True) * inv
    return c * jax.lax.rsqrt(v + 1e-5)


def _after(w, token):
    if token is None:
        return w
    head = pltpu.bitcast(pltpu.bitcast(w[0:16], U32) | token, BF16)
    return jnp.concatenate([head, w[16:]], 0)


def _dft_constants(S, D, FP):
    nf = D // 2 + 1
    d = np.arange(D)[:, None]
    k = np.arange(nf)[None, :]
    ang = 2.0 * np.pi * ((d * k) % D) / D
    cos, sin = np.cos(ang), np.sin(ang)
    n0 = FP - LANE
    ck = np.full((nf,), 2.0)
    ck[0] = ck[D // 2] = 1.0

    def pack(re, im):
        return np.concatenate(
            [re[:, :n0], re[:, D // 2:], im[:, 1:n0], re[:, n0:D // 2], im[:, n0:D // 2]], 1)

    fwd = pack(cos, -sin)
    inv = pack(cos * ck / D, -sin * ck / D).T
    k1 = np.arange(R)[:, None, None]
    k2 = np.arange(LANE)[None, :, None]
    n2 = np.arange(LANE)[None, None, :]
    a = 2.0 * np.pi * ((n2 * (k1 + R * k2)) % S) / S
    c, s = np.cos(a), np.sin(a)
    g = np.concatenate([np.concatenate([c, s], 2), np.concatenate([-s, c], 2)], 1)
    gi = np.transpose(g, (0, 2, 1)) / S
    slab = lambda m: np.ascontiguousarray(
        m.reshape(m.shape[0], -1, LANE).transpose(1, 0, 2)).astype(BF16)
    return slab(fwd), slab(inv), g.astype(BF16), gi.astype(BF16)


def _fft4(x, sign):
    (ar, ai), (br, bi), (cr, ci), (dr, di) = x
    sr, si, tr, ti = ar + cr, ai + ci, ar - cr, ai - ci
    ur, ui, vr, vi = br + dr, bi + di, br - dr, bi - di
    p, m = (tr - vi, ti + vr), (tr + vi, ti - vr)
    y1, y3 = (p, m) if sign > 0 else (m, p)
    return [(sr + ur, si + ui), y1, (sr - ur, si - ui), y3]


def _twiddle16(z, e, sign):
    r, i = z
    if e == 0:
        return z
    if e == 4:
        return (-i, r) if sign > 0 else (i, -r)
    c = float(np.cos(2 * np.pi * e / 16))
    s = float(sign * np.sin(2 * np.pi * e / 16))
    if e % 4 == 2:
        sg = s / c
        return ((r - i) * c, (i + r) * c) if sg > 0 else ((r + i) * c, (i - r) * c)
    return (r * c - i * s, i * c + r * s)


def _fft16(x, sign):
    t = [_fft4([x[b + 4 * a] for a in range(4)], sign) for b in range(4)]
    y = [None] * 16
    for k1 in range(4):
        o = _fft4([_twiddle16(t[b][k1], b * k1, sign) for b in range(4)], sign)
        for k2 in range(4):
            y[k1 + 4 * k2] = o[k2]
    return y


def _kernel(x_hbm, mem_hbm, wq_hbm, wk_hbm, wv_hbm, wo_hbm, wr_hbm, wi_hbm,
            fd_hbm, fi_hbm, g_hbm, gi_hbm, out_hbm,
            xin, xb, mem0, stage, wqkv, wo, wrb, wib, wrf, wif, fd, fi, g, gi,
            x, hbuf, oc, otok, fill, xa, ya, bufa, bufb, bufc, bufd, ob, sems, *, S, D, H, M, SEG, FP):
    L = M + SEG
    nseg = S // SEG
    ND = D // LANE
    NF = FP // LANE
    nf = D // 2 + 1
    G = LANE // L
    groups = [list(range(a, min(a + G, H))) for a in range(0, H, G)]
    scale = LANE ** -0.5
    UA = 3
    CH = 8 * SEG
    assert (nseg - 1) % UA == 0 and (UA + 2) * SEG <= CH

    rows = LANE * H // 2
    cp_x = pltpu.make_async_copy(x_hbm.at[0:CH], xb.at[0:CH], sems.at[0])
    cp_x2 = pltpu.make_async_copy(x_hbm.at[CH:S], xin.at[CH:S], sems.at[0])
    cp_mem = pltpu.make_async_copy(mem_hbm, mem0, sems.at[1])
    cp_w = [pltpu.make_async_copy(w.bitcast(U32).at[pl.ds(c * rows, rows)], stage.at[i * ND + c, 0:rows],
                                  sems.at[2 + i * ND + c])
            for i, w in enumerate((wq_hbm, wk_hbm, wv_hbm)) for c in range(ND)]
    n = 2 + 3 * ND
    cp_wo = [pltpu.make_async_copy(wo_hbm.bitcast(U32).at[:, pl.ds(c * LANE, LANE)], wo.at[c], sems.at[n + c])
             for c in range(ND)]
    n += ND
    cp_b = [pltpu.make_async_copy(a, b, sems.at[n + i]) for i, (a, b) in enumerate(
        ((wr_hbm, wrb), (wi_hbm, wib), (fd_hbm, fd), (fi_hbm, fi), (g_hbm, g), (gi_hbm, gi)))]
    n_out = n + len(cp_b)
    queue = cp_w + cp_wo
    DEPTH = 4
    for cp in [cp_x, cp_mem] + queue[:DEPTH]:
        cp.start()

    r = jax.lax.broadcasted_iota(jnp.int32, fill.shape, 0)
    c = jax.lax.broadcasted_iota(jnp.int32, fill.shape, 1)
    rb = sum((r >= L * j).astype(jnp.int32) for j in range(1, G + 1))
    cb = sum((c >= L * j).astype(jnp.int32) for j in range(1, G + 1))
    ri, ci = r - L * rb, c - L * cb
    fill[...] = jnp.where(rb == cb, jnp.where((ri < M) | (ri >= ci), 0.0, -1e9),
                          -jnp.inf).astype(F32)
    otok[...] = jnp.zeros(otok.shape, F32)

    cp_x.wait()
    x[0:CH, :] = xb[0:CH, :].astype(F32)
    cp_mem.wait()

    for t, cp in enumerate(cp_w):
        cp.wait()
        queue[t + DEPTH].start()
        i, c = divmod(t, ND)

        @pl.loop(0, H // 2)
        def _(j):
            w = stage[t, pl.ds(j, LANE, stride=H // 2), :]
            lo = pltpu.bitcast(w << 16, F32).astype(BF16)
            hi = pltpu.bitcast(w & np.uint32(0xFFFF0000), F32).astype(BF16)
            wqkv[i * H + 2 * j, c * LANE // 2:(c + 1) * LANE // 2, :] = pltpu.bitcast(lo, U32)
            wqkv[i * H + 2 * j + 1, c * LANE // 2:(c + 1) * LANE // 2, :] = pltpu.bitcast(hi, U32)

    for cp in queue[len(cp_w) + DEPTH:]:
        cp.start()

    def token(zero, *vals):
        bits = functools.reduce(jnp.bitwise_or, [pltpu.bitcast(v, U32) for v in vals])
        return bits & zero.astype(U32)

    def finish_segment(s):
        r0 = pl.multiple_of(s * SEG, SEG)
        xn = x[pl.ds(r0, SEG), :] + otok[...]
        x[pl.ds(r0, SEG), :] = xn
        ln = _layernorm(xn)
        xb[pl.ds(r0, SEG), :] = ln.astype(BF16)
        return ln

    def a_step(s, before_out_proj=None):
        st = {}

        def proj(i, hd):
            st[i, hd] = _dot(hbuf[...], _after(pltpu.bitcast(wqkv[i * H + hd], BF16), st.pop(('tok', slot), None)))

        def scores(gi_):
            gr = groups[gi_]
            pad = [jnp.zeros((LANE - L * len(gr), LANE), F32)]
            q = jnp.concatenate([st.pop((0, hd)) for hd in gr], 0)
            k = jnp.concatenate([st.pop((1, hd)) for hd in gr] + pad, 0).astype(BF16)
            st['v', gi_] = jnp.concatenate([st.pop((2, hd)) for hd in gr] + pad, 0).astype(BF16)
            st['s', gi_] = _dot_nt(q, k)

        def softmax(gi_):
            f = fill[0:L * len(groups[gi_]), :]
            sc = jnp.where(f < 0.0, f, st.pop(('s', gi_)) * scale)
            e = jnp.exp(sc - jnp.max(sc, axis=1, keepdims=True))
            st['p', gi_] = e / jnp.sum(e, axis=1, keepdims=True)

        def values(gi_):
            o = _dot(st.pop(('p', gi_)), st.pop(('v', gi_)))
            for j, hd in enumerate(groups[gi_]):
                oc[:, hd * LANE:(hd + 1) * LANE] = o[L * j:L * (j + 1)]
            done.update(groups[gi_])

        def out_proj(h0, h1):
            a, b = h0 * LANE, h1 * LANE
            tok = st.pop(('tok', slot), None)
            t = jnp.concatenate(
                [_dot(oc[:, a:b], _after(pltpu.bitcast(wo[c, a // 2:b // 2, :], BF16), tok if c == 0 else None))
                 for c in range(ND)], 1)
            st['acc'] = st['acc'] + t if 'acc' in st else t

        def next_ln(_):
            r1 = pl.multiple_of(jnp.minimum(s + 1, nseg - 1) * SEG, SEG)
            ln = _layernorm(x[pl.ds(r1, SEG), :])
            hbuf[M:L, :] = ln
            st['tok', 3 * H + 24] = token(
                s >> 16, *[ln[a:a + 8, D - LANE:] for a in range(0, SEG, 8)])

        def prev_finish(_):
            ln = finish_segment(jnp.maximum(s - 1, 0))
            st['tok', 11] = token(s >> 16, *[ln[a:a + 8, D - LANE:] for a in range(0, SEG, 8)])

        events, done = {}, set()
        for gi_, gr in enumerate(groups):
            last = 3 * (gr[-1] + 1) - 1
            for delay, fn in ((0, scores), (3, softmax), (9, values)):
                events.setdefault(last + delay, []).append((fn, gi_))
        events.setdefault(0, []).append((prev_finish, 0))
        events.setdefault(3 * H + 16, []).append((next_ln, 0))
        slot = 0

        def tick():
            nonlocal slot
            for fn, a in events.pop(slot, []):
                fn(a)
            slot += 1

        for gr in groups:
            for i in (1, 0, 2):
                for hd in gr:
                    proj(i, hd)
                    tick()
        WC = 4
        if before_out_proj is not None:
            before_out_proj()
        for h0 in range(0, H, WC):
            while not done.issuperset(range(h0, h0 + WC)):
                tick()
            out_proj(h0, h0 + WC)
            for _ in range(WC):
                tick()
        assert not events and set(st) == {'acc'}
        hbuf[0:M, :] = st['acc'][0:M]
        otok[...] = st['acc'][M:L]

    def layer_a(layer):
        hbuf[0:M, :] = mem0[...].astype(F32)
        hbuf[M:L, :] = _layernorm(x[0:SEG, :])

        def wait_wo():
            @pl.when(layer == 0)
            def _():
                for cp in cp_wo:
                    cp.wait()
                cp_x2.start()

        a_step(layer >> 8, wait_wo)

        @pl.loop(0, (nseg - 1) // UA)
        def _(j):
            @pl.when((layer == 0) & (j == 1))
            def _():
                cp_x2.wait()
                for cp in cp_b:
                    cp.start()

                @pl.loop(1, S // CH)
                def _(i):
                    rs = pl.ds(pl.multiple_of(i * CH, CH), CH)
                    x[rs, :] = xin[rs, :].astype(F32)

            for u in range(UA):
                a_step(1 + j * UA + u)

        finish_segment(nseg - 1)
        otok[...] = jnp.zeros(otok.shape, F32)

    RC = 16
    NCH = LANE // RC

    def chunk_rows(i, n1):
        return pl.ds(n1 * LANE + i * RC, RC)

    lane = jax.lax.broadcasted_iota(jnp.int32, (8, LANE), 1)
    HALF = LANE // 2
    IM0, MIX = NF - 1, 2 * NF - 2

    def dft_fwd(i, buf):
        xh = jnp.concatenate([xb[chunk_rows(i, n1), :] for n1 in range(R)], 0)
        for c in [c_ + o for c_ in range(NF - 1) for o in (0, IM0)] + [MIX]:
            buf[c] = _dot(xh, _after(fd[c], (yield)))

    def radix_fwd(i, buf, zero):
        for c in range(NF):
            for h in range(0, RC, 8):
                def load(n1):
                    rs = slice(n1 * RC + h, n1 * RC + h + 8)
                    if c < NF - 1:
                        im = buf[IM0 + c, rs, :]
                        return buf[c, rs, :], jnp.where(lane == 0, 0.0, im) if c == 0 else im
                    t = buf[MIX, rs, :]
                    u = pltpu.roll(jnp.where(lane == 0, buf[IM0, rs, :], t), HALF, 1)
                    return jnp.where(lane == HALF, u, t), jnp.where(lane == HALF, 0.0, u)

                r0 = i * RC + h
                for k1, (re, im) in enumerate(_fft16([load(n1) for n1 in range(R)], -1)):
                    ya[c, k1, pl.ds(r0, 8), :] = re
                    ya[c, k1, pl.ds(LANE + r0, 8), :] = im
            yield ya[c, 0, pl.ds(pl.multiple_of(i * RC + zero, 8), 8), :]

    def filter_transpose(i):
        n_ = S // NCH
        cols = pl.ds(i * n_, n_)
        for c in range(NF):
            for src, dst in ((wrb, wrf), (wib, wif)):
                lo, hi = c * LANE, min((c + 1) * LANE, nf)
                t = src[lo:hi, cols].astype(F32)
                if hi - lo < LANE:
                    t = jnp.concatenate([t, jnp.zeros((LANE - (hi - lo), n_), F32)], 0)
                t = t.T
                dst[c, cols, :] = t
            yield t[n_ - 8:]

    def radix_inv(i, buf, zero):
        for c in range(NF):
            for h in range(0, RC, 8):
                r0 = i * RC + h
                v = [(xa[c, k1, pl.ds(r0, 8), :], xa[c, k1, pl.ds(LANE + r0, 8), :])
                     for k1 in range(R)]
                o = _fft16(v, +1)
                rs = slice(h * R, (h + 8) * R)
                re = jnp.concatenate([z[0] for z in o], 0)
                im = jnp.concatenate([z[1] for z in o], 0)
                if c < NF - 1:
                    buf[c, rs, :] = re.astype(BF16)
                    buf[IM0 + c, rs, :] = im.astype(BF16)
                else:
                    ln = jax.lax.broadcasted_iota(jnp.int32, re.shape, 1)
                    u = pltpu.roll(jnp.where(ln == HALF, re, im), HALF, 1)
                    buf[MIX, rs, :] = jnp.where(ln < HALF, re, u).astype(BF16)
                    buf[IM0, rs, :] = jnp.where(
                        ln == 0, u, buf[IM0, rs, :].astype(F32)).astype(BF16)
            yield buf[0, pl.ds(pl.multiple_of(zero, 16), 16), :]

    def out_copy(i):
        rs = pl.ds(i * RC, RC)
        return pltpu.make_async_copy(ob.at[i], out_hbm.at[:, rs, :], sems.at[n_out + i])

    def dft_inv(i, buf):
        zz = jnp.concatenate([buf[c] for c in range(ND)], 1)
        for c in range(ND):
            y = _dot(zz, _after(fi[c], (yield)))
            cs = slice(c * LANE, (c + 1) * LANE)
            for n1 in range(R):
                xn = x[chunk_rows(i, n1), cs] + jnp.concatenate(
                    [y[h * R + n1 * 8:h * R + n1 * 8 + 8] for h in range(0, RC, 8)], 0)
                x[chunk_rows(i, n1), cs] = xn
                ob[i, n1, :, cs] = xn.astype(BF16)

    def overlap(zero, mxu, *vpu):
        LAG = 2
        next(mxu)
        toks = [None] * LAG
        while True:
            vals = [v for v in (next(gen, None) for gen in vpu) if v is not None]
            toks.append(token(zero, *vals) if vals else None)
            try:
                mxu.send(toks.pop(0))
            except StopIteration:
                break

    def layer_b(layer):
        zero = layer >> 8
        bufs = (bufa, bufb)
        overlap(zero, dft_fwd(0, bufa), filter_transpose(0))
        for i in range(1, NCH):
            overlap(zero, dft_fwd(i, bufs[i % 2]), radix_fwd(i - 1, bufs[1 - i % 2], zero),
                    filter_transpose(i))
        list(radix_fwd(NCH - 1, bufb, zero))
        U = 8

        @pl.loop(0, R // U)
        def _(j):
            items = [(j * U + u, c) for u in range(U) for c in range(NF)]
            z = {}
            for t in range(len(items) + 3):
                if t < len(items):
                    k1, c = items[t]
                    z[t] = _dot(g[k1], ya[c, k1].astype(BF16))
                if t >= 3:
                    k1, c = items[t - 3]
                    zt = z.pop(t - 3)
                    zr, zi = zt[0:LANE], zt[LANE:]
                    wr = wrf[c, pl.ds(k1, LANE, stride=R), :]
                    wi = wif[c, pl.ds(k1, LANE, stride=R), :]
                    zz = jnp.concatenate([zr * wr - zi * wi, zr * wi + zi * wr], 0)
                    xa[c, k1] = _dot(gi[k1], zz.astype(BF16))

        @pl.when(layer == 1)
        def _():
            for i in range(NCH):
                out_copy(i).wait()

        bufs = (bufc, bufd)
        list(radix_inv(0, bufc, zero))
        for i in range(NCH):
            nxt = [radix_inv(i + 1, bufs[1 - i % 2], zero)] if i + 1 < NCH else []
            overlap(zero, dft_inv(i, bufs[i % 2]), *nxt)
            out_copy(i).start()

    @pl.loop(0, 2)
    def _(layer):
        layer_a(layer)

        @pl.when(layer == 0)
        def _():
            for cp in cp_b:
                cp.wait()

        layer_b(layer)

    for i in range(NCH):
        out_copy(i).wait()


@functools.partial(jax.jit, static_argnames=("A_seg_len",))
def pallas_interleave_layers__memory_aug_recurrent_mem_tr__spectral_gfnet__prompt_kernel(
    A_x, A_mem0, A_Wq, A_Wk, A_Wv, A_Wo, A_seg_len, B_x, B_w_r, B_w_i,
):
    del B_x
    B, S, D = A_x.shape
    _, H, Dh = A_Wq.shape
    M = A_mem0.shape[1]
    SEG = int(A_seg_len)
    nf = D // 2 + 1
    FP = -(-nf // LANE) * LANE
    L = M + SEG
    assert B == 1 and Dh == LANE and S == R * LANE and D % LANE == 0 and S % SEG == 0
    assert M % 8 == 0 and SEG % 16 == 0 and L <= LANE and H % 4 == 0 and D // LANE % 2 == 1
    ND, NF = D // LANE, FP // LANE
    consts = _dft_constants(S, D, FP)

    vm = pltpu.VMEM
    scratch = [
        vm((S, D), BF16),
        vm((S, D), BF16),
        vm((M, D), BF16),
        vm((3 * ND, (LANE + 1) * H // 2, LANE), U32),
        vm((3 * H, D // 2, LANE), U32),
        vm((ND, H * Dh // 2, LANE), U32),
        vm((nf, S), BF16), vm((nf, S), BF16),
        vm((NF, S + R, LANE), F32), vm((NF, S + R, LANE), F32),
        vm(consts[0].shape, BF16), vm(consts[1].shape, BF16),
        vm(consts[2].shape, BF16), vm(consts[3].shape, BF16),
        vm((S, D), F32),
        vm((L, D), F32),
        vm((L, H * Dh), F32),
        vm((SEG, D), F32),
        vm((LANE // L * L, LANE), F32),
        vm((NF, R, 2 * LANE, LANE), F32),
        vm((NF, R, 2 * LANE, LANE), F32),
        vm((ND, R * 16, LANE), F32),
        vm((ND, R * 16, LANE), F32),
        vm((ND, R * 16, LANE), BF16),
        vm((ND, R * 16, LANE), BF16),
        vm((LANE // 16, R, 16, D), BF16),
        pltpu.SemaphoreType.DMA((2 + 4 * ND + 6 + LANE // 16,)),
    ]
    any_spec = pl.BlockSpec(memory_space=pltpu.HBM)
    out = pl.pallas_call(
        functools.partial(_kernel, S=S, D=D, H=H, M=M, SEG=SEG, FP=FP),
        out_shape=jax.ShapeDtypeStruct((R, LANE, D), BF16),
        in_specs=[any_spec] * 12,
        out_specs=any_spec,
        scratch_shapes=scratch,
        compiler_params=pltpu.CompilerParams(vmem_limit_bytes=110 * 2**20),
    )(A_x.reshape(S, D), A_mem0.reshape(M, D),
      A_Wq.reshape(D * H, Dh), A_Wk.reshape(D * H, Dh), A_Wv.reshape(D * H, Dh),
      A_Wo.reshape(H * Dh, D), B_w_r.T, B_w_i.T, *consts)
    return out.reshape(B, S, D)
```
